```python
import os as _os
_os.environ.setdefault("JAX_PLATFORMS", "cpu")
import jax
import jax.numpy as jnp

def _softmax(x, axis=-1):
    return jax.nn.softmax(x, axis=axis)
def _gelu(x):
    return jax.nn.gelu(x, approximate=True)
def _silu(x):
    return jax.nn.silu(x)
def _sigmoid(x):
    return jax.nn.sigmoid(x)
def _layernorm(x, axis=-1, eps=1e-5):
    m = jnp.mean(x, axis=axis, keepdims=True)
    v = jnp.var(x, axis=axis, keepdims=True)
    return (x - m) / jnp.sqrt(v + eps)
def _scatter_add(tgt, idx, src, axis=0):
    return tgt.at[idx].add(src)
def _segment_sum(src, seg, n):
    return jax.ops.segment_sum(src, seg, n)
class _Rng:
    def __init__(self, key):
        self._k = key
    def _next(self):
        self._k, sub = jax.random.split(self._k)
        return sub
    def normal(self, shape):
        return jax.random.normal(self._next(), shape, dtype=jnp.bfloat16)
    def randint(self, lo, hi, shape):
        return jax.random.randint(self._next(), shape, lo, hi, dtype=jnp.int32)
    def uniform(self, shape, lo=0.0, hi=1.0):
        return jax.random.uniform(self._next(), shape, jnp.bfloat16, lo, hi)
    def permutation(self, n):
        return jax.random.permutation(self._next(), n)


kernel_name = 'gated_mix__sliding_local_dilated__moe_arch_mod__prompt'

def setup_inputs():
    _rng = _Rng(jax.random.key(int.from_bytes(__import__("os").urandom(4), "little")))
    _w = (lambda a: (lambda t: t.astype(jnp.bfloat16) if jnp.issubdtype(t.dtype, jnp.floating) else t)(jnp.asarray(a)))
    def _A_setup():
        B, S, D = 1, 2048, 640
        return {
            "x": _w((lambda *s: _rng.normal(s) * 0.05)(B, S, D)),
            "wqkv": _w((lambda *s: _rng.normal(s) * 0.8)(D, 3 * D)),
            "wo": _w((lambda *s: _rng.normal(s) * 0.05)(D, D)),
        }
    _A_in = _A_setup()

    def _B_setup():
        B, S, D, F, C = 1, 2048, 640, 1728, 1
        return {
            "x": _w((lambda *s: _rng.normal(s) * 0.05)(B, S, D)),
            "w_r": _w((lambda *s: _rng.normal(s) * 1.6)(D)),
            "w_gate": _w((lambda *s: _rng.normal(s) * 0.4)(D, F)),
            "w_up": _w((lambda *s: _rng.normal(s) * 0.4)(D, F)),
            "w_down": _w((lambda *s: _rng.normal(s) * 0.4)(F, D)),
        }
    _B_in = _B_setup()

    return {
        "A_x": _A_in["x"],
        "A_wqkv": _A_in["wqkv"],
        "A_wo": _A_in["wo"],
        "B_x": _B_in["x"],
        "B_w_r": _B_in["w_r"],
        "B_w_gate": _B_in["w_gate"],
        "B_w_up": _B_in["w_up"],
        "B_w_down": _B_in["w_down"],
        "gate_w": _w((lambda *s: _rng.normal(s) * 0.05)(640) * 16.0),
    }

def reference(A_x, A_wqkv, A_wo, B_x, B_w_r, B_w_gate, B_w_up, B_w_down, gate_w):
    def _A_ref(x, wqkv, wo):
        B, S, D = x.shape
        H = 32; Dh = D // H
        W, dil = 8, 2
        qkv = (lambda x, *d: x.transpose(*d))((x @ wqkv).reshape(B, S, 3, H, Dh), 2, 0, 3, 1, 4)
        q, k, v = qkv[0], qkv[1], qkv[2]
        scale = Dh ** -0.5
        pos = jnp.arange(S)
        off = jnp.arange(W) * dil
        idx = pos[:, None] - off[None, :]
        mask = idx >= 0
        idx_c = jnp.where(mask, idx, 0).reshape(-1)
        kg = k[:, :, idx_c, :].reshape(B, H, S, W, Dh)
        vg = v[:, :, idx_c, :].reshape(B, H, S, W, Dh)
        logits = jnp.einsum("bhsd,bhswd->bhsw", q, kg) * scale
        logits = jnp.where(mask[None, None, :, :], logits, -1e9)
        attn = _softmax(logits, axis=-1)
        o = jnp.einsum("bhsw,bhswd->bhsd", attn, vg)
        return (lambda x, *d: x.transpose(*d))(o, 0, 2, 1, 3).reshape(B, S, D) @ wo

    def _B_ref(x, w_r, w_gate, w_up, w_down):
        B, S, D = x.shape
        C = 1
        r = x @ w_r
        idx = jnp.argsort(-r, axis=-1)[:, :C]
        idx_e = jnp.repeat(idx.reshape(B, C, 1), D, axis=2)
        x_sel = jnp.take_along_axis(x, idx_e, axis=1)
        g = _silu(x_sel @ w_gate)
        u = x_sel @ w_up
        y = (g * u) @ w_down
        r_sel = _sigmoid(jnp.take_along_axis(r, idx, axis=1))
        y = y * r_sel.reshape(B, C, 1)
        b_off = (jnp.arange(B) * S).reshape(B, 1)
        flat_idx = (idx + b_off).reshape(B * C)
        zero = (x * 0.0).reshape(B * S, D)
        upd = _scatter_add(zero, flat_idx, y.reshape(B * C, D), axis=0)
        return x + upd.reshape(B, S, D)

    x = A_x
    g = _sigmoid((x * gate_w).sum(-1, keepdims=True))
    a = _A_ref(x, A_wqkv, A_wo)
    b = _B_ref(x, B_w_r, B_w_gate, B_w_up, B_w_down)
    return g * a + (1 - g) * b
```

```python
import functools

import jax
import jax.numpy as jnp
import numpy as np
import jax.experimental.pallas as pl
import jax.experimental.pallas.tpu as pltpu

S = 2048
D = 640
H = 32
DH = 20
NW = 8
DIL = 2
F = 1728
LT = D // 128
HALO = 16
LOG2E = 1.4426950408889634
CQ = (DH ** -0.5) * LOG2E
NEG = -1e9 * LOG2E

_NT = (((1,), (1,)), ((), ()))

CFG = dict(
    C=128,
    CC=128,
    tail_rows=128,
    tail_cc=64,
    R=16,
    a_tiles=3,
    xa=256,
    xb=128,
    xc=1152,
    late_wait=30,
    gap=6,
    first=3,
    w_b=1.4, w_p=1.0, w_f=1.4,
    w_c=0.0,
    fine=True,
    c_slack=0.5,
    b_slack=4,
    b_behind=300,
    fence_lag=2,
    p_ahead=128,
    router_gap=8,
    paced=True,
    out_splits=(1920,),
)


def _sigmoid(z):
    return 0.5 * jnp.tanh(0.5 * z) + 0.5


def _interleave(a, b):
    ev = (a & jnp.uint32(0xFFFF)) | (b << 16)
    od = (a >> 16) | (b & jnp.uint32(0xFFFF0000))
    return ev, od


def _kernel(x_hbm, w_hbm, wo_hbm, wr_hbm, wg_hbm, wu_hbm, wd_hbm, gw_hbm,
            out_hbm,
            x_vm, w_raw, tscr, wp, wo_raw, wo_u32, wo_p, wr_vm, gw_vm,
            wg_vm, wu_vm, wd_vm, qkv, obuf, out_vm, g_vm,
            sems, *, cfg):
    C, R = cfg["C"], cfg["R"]
    NC = S // C
    XA, XB = cfg["xa"], cfg["xb"]
    M0 = XA + XB
    xs = (0, XA, M0, cfg["xc"], S)
    f32 = jnp.float32
    bf16 = jnp.bfloat16
    u32 = jnp.uint32

    def x_copy(i):
        return pltpu.make_async_copy(
            x_hbm.at[0, pl.ds(xs[i], xs[i + 1] - xs[i]), :],
            x_vm.at[pl.ds(xs[i], xs[i + 1] - xs[i]), :], sems.at[i])

    def w_copy(kk):
        return pltpu.make_async_copy(
            w_hbm.at[pl.ds(kk * 128, 128), :],
            w_raw.at[pl.ds(kk * 128, 128), :], sems.at[4 + kk])

    misc = [
        pltpu.make_async_copy(wr_hbm, wr_vm, sems.at[9]),
        pltpu.make_async_copy(gw_hbm, gw_vm, sems.at[10]),
        pltpu.make_async_copy(wo_hbm, wo_raw, sems.at[11]),
        pltpu.make_async_copy(wg_hbm, wg_vm, sems.at[12]),
        pltpu.make_async_copy(wu_hbm, wu_vm, sems.at[13]),
        pltpu.make_async_copy(wd_hbm, wd_vm, sems.at[14]),
    ]

    def out_copy(slot, r0, r1):
        return pltpu.make_async_copy(
            out_vm.at[pl.ds(r0, r1 - r0), :],
            out_hbm.at[0, pl.ds(r0, r1 - r0), :], sems.at[15 + slot])

    def wait(cp, name):
        if cfg.get("scopes"):
            with jax.named_scope("wait_" + name):
                cp.wait()
        else:
            cp.wait()

    w_copy(0).start()
    x_copy(0).start()
    w_copy(1).start()
    x_copy(1).start()
    w_copy(2).start()
    w_copy(3).start()
    w_copy(4).start()
    misc[0].start()
    misc[1].start()
    x_copy(2).start()
    misc[2].start()
    x_copy(3).start()
    misc[3].start()
    misc[4].start()
    misc[5].start()

    qkv[LT:3 * LT, 0:HALO, :] = jnp.zeros((2 * LT, HALO, 128), f32)

    def permute_w(kk):
        for t in range(3):
            for c in range(LT):
                tile = w_raw[kk * 128:(kk + 1) * 128,
                             t * D + c * 128:t * D + (c + 1) * 128]
                tscr[kk, t, c * 64:(c + 1) * 64, :] = pltpu.bitcast(tile.T, u32)
        for t in range(3):
            for dp in range(DH // 2):
                a = tscr[kk, t, pl.ds(dp, 16, stride=DH // 2), :]
                b = tscr[kk, t, pl.ds(160 + dp, 16, stride=DH // 2), :]
                ev, od = _interleave(a, b)
                r0 = (t * D + 2 * dp * 32) // 2
                wp[r0:r0 + 16, kk * 128:(kk + 1) * 128] = ev
                wp[r0 + 16:r0 + 32, kk * 128:(kk + 1) * 128] = od

    def permute_wo():
        for c in range(LT):
            wo_u32[c] = pltpu.bitcast(wo_raw[:, c * 128:(c + 1) * 128], u32)
        for c in range(LT):
            for dp in range(DH // 2):
                a = wo_u32[c, pl.ds(dp, 16, stride=DH // 2), :]
                b = wo_u32[c, pl.ds(160 + dp, 16, stride=DH // 2), :]
                ev, od = _interleave(a, b)
                r0 = dp * 32
                wo_p[r0:r0 + 16, c * 128:(c + 1) * 128] = ev
                wo_p[r0 + 16:r0 + 32, c * 128:(c + 1) * 128] = od

    def mm_part(r0, r1, kk):
        for s0 in range(r0, r1, C):
            w = pltpu.bitcast(wp[:, kk * 128:(kk + 1) * 128], bf16)
            y = jax.lax.dot_general(x_vm[s0:s0 + C, kk * 128:(kk + 1) * 128], w, _NT,
                                    preferred_element_type=f32)
            for j in range(3 * LT):
                blk = y[:, j * 128:(j + 1) * 128]
                if kk > 0:
                    blk = blk + qkv[j, HALO + s0:HALO + s0 + C, :]
                qkv[j, HALO + s0:HALO + s0 + C, :] = blk

    wait(w_copy(0), "w0")
    permute_w(0)
    wait(x_copy(0), "x0")
    mm_part(0, XA // 2, 0)
    wait(w_copy(1), "w1")
    permute_w(1)
    mm_part(XA // 2, XA, 0)
    mm_part(0, XA, 1)
    wait(x_copy(1), "x1")
    wait(w_copy(2), "w2")
    permute_w(2)
    mm_part(XA, M0, 0)
    mm_part(XA, M0, 1)
    mm_part(0, M0 - 128, 2)
    wait(w_copy(3), "w3")
    wait(w_copy(4), "w4")
    permute_w(3)
    permute_w(4)
    mm_part(M0 - 128, M0, 2)
    mm_part(0, M0, 3)
    mm_part(0, M0, 4)

    wait(misc[0], "wr")
    wait(misc[1], "gw")
    wait(x_copy(2), "x2")
    wait(misc[2], "wo")

    def tiles8(v):
        return [jnp.broadcast_to(v[:, j * 128:(j + 1) * 128], (8, 128)) for j in range(LT)]

    wr = tiles8(wr_vm[...].astype(f32)[None, :])
    gw = tiles8(gw_vm[...].astype(f32)[None, :])

    zero = jax.lax.shift_right_logical(
        jnp.max(jax.lax.shift_right_logical(pltpu.bitcast(wr[0], jnp.int32), 16)), 16)
    zvec = pltpu.bitcast(jnp.full((8, 128), zero, jnp.int32), u32)
    z16 = pl.multiple_of(zero * 16, 16)

    def token(vals):
        u = None
        for v in vals:
            if v.dtype != u32:
                v = pltpu.bitcast(v, u32)
            for r in range(0, v.shape[0], 8):
                u = v[r:r + 8] if u is None else u | v[r:r + 8]
        return u & zvec

    def tied(v, tok):
        if tok is None:
            return v
        if v.dtype == u32:
            return v | tok
        return pltpu.bitcast(pltpu.bitcast(v, u32) | tok, v.dtype)

    def tie_tiles(ref, r0, ng, tok_of):
        parts, prev = [], r0
        for g in range(ng):
            tk = [tok_of(g, c) for c in range(LT)]
            if all(t is None for t in tk):
                continue
            r = r0 + g * 64
            if r > prev:
                parts.append(ref[prev:r, :])
            parts.append(jnp.concatenate(
                [tied(ref[r:r + 8, c * 128:(c + 1) * 128], tk[c]) for c in range(LT)], axis=1))
            prev = r + 8
        parts.append(ref[prev:r0 + 64 * ng, :])
        return parts[0] if len(parts) == 1 else jnp.concatenate(parts, axis=0)

    NTA = cfg["a_tiles"]

    def unit_a(s0, xc, u, toks):
        w = tie_tiles(wp, u * NTA * 64, NTA, lambda n, kk: toks.get((n, kk)))
        y = jax.lax.dot_general(xc, pltpu.bitcast(w, bf16), _NT, preferred_element_type=f32)
        for j in range(NTA):
            qkv[u * NTA + j, HALO + s0:HALO + s0 + C, :] = y[:, j * 128:(j + 1) * 128]
        return [y[0:8, j * 128:(j + 1) * 128] for j in range(NTA)]

    def attn_block(s0, rel):
        r0 = HALO + s0
        cq = tied(jnp.full((8, 128), CQ, f32), rel)
        q = [(qkv[j, r0:r0 + R, :].reshape(R // 8, 8, 128) * cq[None]).reshape(R, 128)
             for j in range(LT)]
        ls = []
        for w in range(NW):
            rw = r0 - DIL * w
            s = q[0] * qkv[LT, rw:rw + R, :]
            for j in range(1, LT):
                s = s + q[j] * qkv[LT + j, rw:rw + R, :]
            l = (s + pltpu.roll(s, 32, 1)) + (pltpu.roll(s, 64, 1) + pltpu.roll(s, 96, 1))
            if s0 < DIL * w:
                row = jax.lax.broadcasted_iota(jnp.int32, (R, 128), 0) + s0
                l = jnp.where(row >= DIL * w, l, NEG)
            ls.append(l)
        m = ls[0]
        for w in range(1, NW):
            m = jnp.maximum(m, ls[w])
        ps = [jnp.exp2(l - m) for l in ls]
        den = ps[0]
        for w in range(1, NW):
            den = den + ps[w]
        inv = pl.reciprocal(den, approx=True)
        inv = inv + inv * (1.0 - den * inv)
        outs = []
        for j in range(LT):
            o = ps[0] * qkv[2 * LT + j, r0:r0 + R, :]
            for w in range(1, NW):
                rw = r0 - DIL * w
                o = o + ps[w] * qkv[2 * LT + j, rw:rw + R, :]
            ob = pltpu.bitcast((o * inv).astype(bf16), u32)
            obuf[s0 // 2:(s0 + R) // 2, j * 128:(j + 1) * 128] = ob
            outs.append(ob)
        return outs

    def unit_c(r0, n, moe, toks):
        o = pltpu.bitcast(obuf[r0 // 2:(r0 + n) // 2, :], bf16)
        w = tie_tiles(wo_p, 0, LT, lambda kk, n: toks.get((n, kk)))
        a = jnp.dot(o, pltpu.bitcast(w, bf16), preferred_element_type=f32)
        g = g_vm[r0:r0 + n, :]
        if moe is not None:
            idx, delta = moe
            row = jax.lax.broadcasted_iota(jnp.int32, (n, 128), 0) + r0
            coef = jnp.where(row == idx, 1.0 - g, 0.0)
        for j in range(LT):
            sl = slice(j * 128, (j + 1) * 128)
            x = x_vm[r0:r0 + n, sl].astype(f32)
            res = x + g * (a[:, sl] - x)
            if moe is not None:
                res = res + coef * delta[j]
            out_vm[r0:r0 + n, sl] = res.astype(bf16)
        return [a[0:8, j * 128:(j + 1) * 128] for j in range(LT)]

    PR = 64

    def rowdot(mat, vec):
        n = mat.shape[0]
        acc = None
        for j in range(LT):
            p = mat[:, j * 128:(j + 1) * 128].reshape(n // 8, 8, 128) * vec[j][None]
            acc = p if acc is None else acc + p
        acc = acc.reshape(n, 128)
        return jnp.broadcast_to(jnp.sum(acc, axis=-1, keepdims=True), (n, 128))

    def pre_block(b, racc, rel):
        lane = jax.lax.broadcasted_iota(jnp.int32, (PR, 128), 1)
        xf = x_vm[b * PR:(b + 1) * PR, :].astype(f32)
        g_vm[b * PR:(b + 1) * PR, :] = _sigmoid(rowdot(xf, [tied(v, rel) for v in gw]))
        return jnp.where(lane == b, rowdot(xf, [tied(v, rel) for v in wr]), racc)

    FB = 64

    def ffn_block(b, xsel, yacc, rel):
        f0 = b * FB
        xr = [tied(v, rel) for v in xsel]
        gt = rowdot(wg_vm[f0:f0 + FB, :].astype(f32), xr)
        up = rowdot(wu_vm[f0:f0 + FB, :].astype(f32), xr)
        h = gt * _sigmoid(gt) * up
        new = []
        for j in range(LT):
            p = wd_vm[f0:f0 + FB, j * 128:(j + 1) * 128].astype(f32) * h
            new.append(yacc[j] + jnp.sum(p.reshape(FB // 8, 8, 128), axis=0))
        return new

    n0 = M0 // C
    racc = jnp.full((PR, 128), -jnp.inf, f32)
    moe = None
    idx = r_sel = tile0 = xsel = yacc = None
    out_copies = []
    out_done = 0
    nfb = F // FB
    npb = S // PR
    CC = cfg["CC"]
    nua = 3 * LT // NTA
    paced = cfg["paced"]

    permute_wo()

    def fence_out():
        return pltpu.bitcast(out_vm[pl.ds(z16, 16), 0:128], u32)

    def fence_g():
        return g_vm[pl.ds(z16, 8), :]

    gap = cfg["gap"]
    a_row, a_unit = M0, 0
    b_row = c_row = 0
    p_blk = f_blk = 0
    x_avail = xs[3]
    qkv_ready = [(M0, -100)]
    b_ready = [(0, -100)]
    slot_out = []
    fence_due = None
    ffn_from = None
    xc = None
    now = 0.0
    busy_until = cfg["first"]
    last_side = False
    k = 0

    def avail(lst, t):
        return max(r for r, u in lst if u <= t)

    while c_row < S:
        if k == cfg["late_wait"]:
            wait(x_copy(3), "x3")
            wait(misc[3], "wg")
            wait(misc[4], "wu")
            wait(misc[5], "wd")
            x_avail = S
            slot_out = []
        cc = CC if c_row < S - cfg["tail_rows"] else cfg["tail_cc"]
        c_ok = (avail(b_ready, now - cfg["c_slack"]) >= c_row + cc
                and p_blk * PR >= c_row + cc)
        if a_row < S and (a_unit > 0 or not c_ok):
            kind, nsl, dur = "a", NTA, 1.0
        elif c_ok:
            kind, nsl, dur = "c", LT, cc / C
        else:
            kind, nsl, dur = "idle", 1, 1.0
        toks = {}
        for sl in range(nsl):
            t = now + sl * dur
            outs = [[] for _ in range(LT)]
            if fence_due is not None and t >= fence_due:
                outs[0].append(fence_out())
                fence_due = None
            if t >= busy_until:
                rels = [v for (u, v) in slot_out if u <= t - gap]
                rel = token([rels[-1]]) if (paced and rels) else None
                p_urgent = p_blk * PR < min(x_avail, b_row + cfg["p_ahead"])
                b_urgent = a_row - b_row > cfg["b_behind"]
                side = (p_blk * PR < x_avail
                        or (ffn_from is not None and t >= ffn_from and f_blk < nfb))
                take_b = (b_row + R <= avail(qkv_ready, t - cfg["b_slack"])
                          and not p_urgent and (b_urgent or not side or last_side))
                last_side = False
                if take_b:
                    for j, ob in enumerate(attn_block(b_row, rel)):
                        outs[j].append(ob)
                    b_row += R
                    b_ready.append((b_row, t))
                    busy_until = max(busy_until, t - 0.99) + cfg["w_b"]
                elif p_blk * PR < x_avail:
                    racc = pre_block(p_blk, racc, rel)
                    for u in range(PR // 8):
                        outs[u * LT // (PR // 8)].append(racc[u * 8:(u + 1) * 8])
                    outs[LT - 1].append(fence_g())
                    p_blk += 1
                    busy_until = max(busy_until, t - 0.99) + cfg["w_p"]
                    last_side = True
                elif side:
                    yacc = ffn_block(f_blk, xsel, yacc, rel)
                    for j in range(LT):
                        outs[j].append(yacc[j])
                    f_blk += 1
                    busy_until = max(busy_until, t - 0.99) + cfg["w_f"]
                    last_side = True
            if not cfg["fine"]:
                outs = [sum(outs, [])] + [[]] * (LT - 1)
            for j in range(LT):
                if outs[j] and paced:
                    toks[(sl, j)] = token(outs[j])
            if kind == "c":
                busy_until += cfg["w_c"] * dur
        if kind == "a":
            assert a_row + C <= x_avail, (a_row, k)
            if a_unit == 0:
                xc = pltpu.bitcast(pltpu.bitcast(x_vm[a_row:a_row + C, :], u32), bf16)
            outs = unit_a(a_row, xc, a_unit, toks)
            a_unit += 1
            if a_unit == nua:
                a_unit = 0
                a_row += C
                qkv_ready.append((a_row, now + nsl * dur))
        elif kind == "c":
            outs = unit_c(c_row, cc, moe, toks)
            c_row += cc
            fence_due = now + nsl * dur + cfg["fence_lag"]
            if moe is not None and (c_row in cfg["out_splits"] or c_row == S):
                cp = out_copy(len(out_copies), out_done, c_row)
                cp.start()
                out_copies.append(cp)
                out_done = c_row
        else:
            outs = []
        slot_out += [(now + j * dur, v) for j, v in enumerate(outs)]
        now += nsl * dur
        if p_blk == npb and idx is None:
            rb = racc.astype(bf16).astype(f32)
            rb = jnp.where(rb != rb, -jnp.inf, rb)
            rmax = jnp.max(rb)
            rowid = (jax.lax.broadcasted_iota(jnp.int32, (PR, 128), 1) * PR
                     + jax.lax.broadcasted_iota(jnp.int32, (PR, 128), 0))
            idx = jnp.min(jnp.where((rowid < S) & (rb == rmax), rowid, S - 1))
            tile0 = pl.multiple_of((idx // 16) * 16, 16)
            r_sel = _sigmoid(jnp.full((1, 128), rmax, f32))
            x16 = x_vm[pl.ds(tile0, 16), :].astype(f32)
            row16 = jax.lax.broadcasted_iota(jnp.int32, (16, D), 0) + tile0
            xsel = tiles8(jnp.sum(jnp.where(row16 == idx, x16, 0.0), axis=0,
                                  keepdims=True))
            yacc = [jnp.zeros((8, 128), f32) for _ in range(LT)]
            ffn_from = now + cfg["router_gap"]
        elif f_blk == nfb and moe is None:
            delta = [jnp.sum(y, axis=0, keepdims=True) * r_sel for y in yacc]
            moe = (idx, delta)
            fix_rows = c_row
            t0 = pl.multiple_of(jnp.minimum(tile0, fix_rows - 16), 16)
            row = jax.lax.broadcasted_iota(jnp.int32, (16, 128), 0) + t0
            coef = jnp.where(row == idx, 1.0 - g_vm[pl.ds(t0, 16), :], 0.0)
            cur = out_vm[pl.ds(t0, 16), :].astype(f32)
            upd = jnp.concatenate([coef * delta[j] for j in range(LT)], axis=1)
            out_vm[pl.ds(t0, 16), :] = (cur + upd).astype(bf16)
            cp = out_copy(len(out_copies), 0, fix_rows)
            cp.start()
            out_copies.append(cp)
            out_done = fix_rows
        if cfg.get("verbose"):
            print(k, kind, dict(a=a_row, b=b_row, c=c_row, p=p_blk, f=f_blk), now)
        k += 1

    assert out_done == S
    for n, cp in enumerate(out_copies):
        wait(cp, "o%d" % n)


def _build(cfg):
    bf16 = jnp.bfloat16
    f32 = jnp.float32
    u32 = jnp.uint32
    hbm_spec = pl.BlockSpec(memory_space=pltpu.MemorySpace.HBM)
    return pl.pallas_call(
        functools.partial(_kernel, cfg=cfg),
        out_shape=jax.ShapeDtypeStruct((1, S, D), bf16),
        in_specs=[hbm_spec] * 8,
        out_specs=hbm_spec,
        scratch_shapes=[
            pltpu.VMEM((S, D), bf16),
            pltpu.VMEM((D, 3 * D), bf16),
            pltpu.VMEM((LT, 3, D // 2, 128), u32),
            pltpu.VMEM((3 * D // 2, D), u32),
            pltpu.VMEM((D, D), bf16),
            pltpu.VMEM((LT, D // 2, 128), u32),
            pltpu.VMEM((D // 2, D), u32),
            pltpu.VMEM((D,), bf16),
            pltpu.VMEM((D,), bf16),
            pltpu.VMEM((F, D), bf16),
            pltpu.VMEM((F, D), bf16),
            pltpu.VMEM((F, D), bf16),
            pltpu.VMEM((3 * LT, HALO + S, 128), f32),
            pltpu.VMEM((S // 2, D), u32),
            pltpu.VMEM((S, D), bf16),
            pltpu.VMEM((S, 128), f32),
            pltpu.SemaphoreType.DMA((15 + len(cfg["out_splits"]) + 2,)),
        ],
        compiler_params=pltpu.CompilerParams(vmem_limit_bytes=100 * 1024 * 1024),
    )


def _call(cfg, A_x, A_wqkv, A_wo, B_w_r, B_w_gate, B_w_up, B_w_down, gate_w):
    return _build(cfg)(A_x, A_wqkv, A_wo, B_w_r, B_w_gate.T, B_w_up.T, B_w_down, gate_w)


@jax.jit
def pallas_gated_mix__sliding_local_dilated__moe_arch_mod__prompt_kernel(
    A_x: jax.Array,
    A_wqkv: jax.Array,
    A_wo: jax.Array,
    B_x: jax.Array,
    B_w_r: jax.Array,
    B_w_gate: jax.Array,
    B_w_up: jax.Array,
    B_w_down: jax.Array,
    gate_w: jax.Array,
):
    del B_x
    return _call(CFG, A_x, A_wqkv, A_wo, B_w_r, B_w_gate, B_w_up, B_w_down, gate_w)
```

```python
import functools

import jax
import jax.numpy as jnp
import jax.experimental.pallas as pl
import jax.experimental.pallas.tpu as pltpu

S = 2048
D = 640
H = 32
DH = 20
NW = 8
DIL = 2
F = 1728
LT = D // 128
HALO = 16
LOG2E = 1.4426950408889634
CQ = (DH ** -0.5) * LOG2E
NEG = -1e9 * LOG2E
C = 128
R = 16
PR = 64
FB = 64

_NT = (((1,), (1,)), ((), ()))

CFG = dict(
    CC=128,
    tail_rows=128,
    tail_cc=64,
    a_passes=5,
    z=(6, 10, 2, 5, 6, 9), cover=3,
    step=0, c_calm=None, rot2=False, stagger=4, pos=(7, 5, 2, 0),
    c_run=99, first_perm=10.4, first_early=12.0, w_p_early=0.8,
    late_t=92,
    gap=5,
    first=2.4,
    quiet=1,
    w_b=1.6, w_p=0.8, w_f=0.8, w_w=0.8, w_b_tail=1.6,
    c_lag=512,
    pv_off=(0.0, 0.2, 0.6, 0.8, 1.2), f_off=(0.0, 0.2, 0.6, 0.8, 1.2), sm_off=None,
    grid=4, phase=0,
    c_slack=0.0,
    b_slack=3,
    b_behind=300,
    fence_lag=3, fence_from=4, w_c=0.0,
    s_w=0.1,
    p_ahead=128,
    router_gap=8,
    tie_f32=False,
    newton=1,
    out_splits=(1664, 1792, 1920, 1984),
)


def _stages(cfg):
    NB = S // C
    xs = lambda js, b0, b1: [("x", j, b0, b1) for j in js]
    w = lambda kk, t0=0, t1=3: ("w", kk, t0, t1)
    na, m0, h, m1, mx, xc = cfg["z"]
    if na:
        head = [
            ([w(0, 0, 1)], []),
            (xs([0], 0, na), [(b, 1, 0, 1) for b in range(na)]),
            ([w(0, 1, 3), ("vec",)] + xs([0], na, m0),
             [(b, 1, 0, 1) for b in range(na, m0)] + [(b, 1) for b in range(m0 - h)]),
        ]
    else:
        head = [
            ([w(0), ("vec",)], []),
            (xs([0], 0, m0), [(b, 1) for b in range(m0 - h)]),
        ]
    return head + [
        ([w(1), w(2)] + xs([1, 2, 3, 4], 0, mx),
         [(b, 1) for b in range(m0 - h, m0)] + [(0, 2), (0, 3)]
         + [(b, 3) for b in range(1, m1 - 1)]),
        ([w(3), w(4)] + (xs([0], m0, xc) if xc > m0 else [])
         + xs([1, 2, 3, 4], mx, xc) + [("wo",)],
         [(m1 - 1, cfg["cover"]), (0, 4)]),
        (xs([0], max(m0, xc), NB) + xs([1, 2, 3, 4], xc, NB) + [("ffn",)], []),
    ]


def _sigmoid(z):
    return 0.5 * jnp.tanh(0.5 * z) + 0.5


def _interleave(a, b):
    ev = (a & jnp.uint32(0xFFFF)) | (b << 16)
    od = (a >> 16) | (b & jnp.uint32(0xFFFF0000))
    return ev, od


def _kernel(x_hbm, w_hbm, wo_hbm, wr_hbm, wg_hbm, wu_hbm, wd_hbm, gw_hbm,
            out_hbm,
            x_vm, w_raw, tscr, wp, wo_raw, wo_u32, wo_p, wr_vm, gw_vm,
            wg_vm, wu_vm, wd_vm, qkv, obuf, out_vm, g_vm,
            sems, *, cfg):
    f32 = jnp.float32
    bf16 = jnp.bfloat16
    u32 = jnp.uint32

    nsem = [0]

    def copy(src, dst):
        nsem[0] += 1
        return pltpu.make_async_copy(src, dst, sems.at[nsem[0] - 1])

    def piece(pc):
        if pc[0] == "x":
            _, j, b0, b1 = pc
            rows = pl.ds(b0 * C, (b1 - b0) * C)
            return [copy(x_hbm.at[0, rows, pl.ds(j * 128, 128)], x_vm.at[j, rows, :])]
        if pc[0] == "w":
            _, kk, t0, t1 = pc
            rows, cols = pl.ds(kk * 128, 128), pl.ds(t0 * D, (t1 - t0) * D)
            return [copy(w_hbm.at[rows, cols], w_raw.at[rows, cols])]
        if pc[0] == "wo":
            return [copy(wo_hbm.at[:, pl.ds(j * 128, 128)], wo_raw.at[j])
                    for j in range(LT)]
        if pc[0] == "vec":
            return [copy(wr_hbm, wr_vm), copy(gw_hbm, gw_vm)]
        assert pc[0] == "ffn"
        return [copy(wg_hbm, wg_vm), copy(wu_hbm, wu_vm), copy(wd_hbm, wd_vm)]

    stages = _stages(cfg)
    stage_cps = [[cp for pc in sg[0] for cp in piece(pc)] for sg in stages]

    def out_copy(r0, r1):
        return [copy(out_vm.at[pl.ds(r0, r1 - r0), :], out_hbm.at[0, pl.ds(r0, r1 - r0), :])]

    def x_lhs(s0, k0, k1):
        cols = [pltpu.bitcast(x_vm[j, s0:s0 + C, :], u32) for j in range(k0, k1)]
        return pltpu.bitcast(cols[0] if len(cols) == 1 else jnp.concatenate(cols, axis=1), bf16)

    def wait(cps, name):
        if cfg.get("scopes"):
            with jax.named_scope("wait_" + name):
                for cp in cps:
                    cp.wait()
        else:
            for cp in cps:
                cp.wait()

    for cps in stage_cps:
        for cp in cps:
            cp.start()

    qkv[LT:3 * LT, 0:HALO, :] = jnp.zeros((2 * LT, HALO, 128), f32)

    def permute_w(kk, t0, t1):
        for t in range(t0, t1):
            for c in range(LT):
                tile = w_raw[kk * 128:(kk + 1) * 128,
                             t * D + c * 128:t * D + (c + 1) * 128]
                tscr[kk, t, c * 64:(c + 1) * 64, :] = pltpu.bitcast(tile.T, u32)
        for t in range(t0, t1):
            for dp in range(DH // 2):
                a = tscr[kk, t, pl.ds(dp, 16, stride=DH // 2), :]
                b = tscr[kk, t, pl.ds(160 + dp, 16, stride=DH // 2), :]
                ev, od = _interleave(a, b)
                r0 = (t * D + 2 * dp * 32) // 2
                wp[r0:r0 + 16, kk * 128:(kk + 1) * 128] = ev
                wp[r0 + 16:r0 + 32, kk * 128:(kk + 1) * 128] = od

    def permute_wo(c):
        wo_u32[c, 0:D // 2, :] = pltpu.bitcast(wo_raw[c], u32)
        outs = []
        for dp in range(DH // 2):
            a = wo_u32[c, pl.ds(dp, 16, stride=DH // 2), :]
            b = wo_u32[c, pl.ds(160 + dp, 16, stride=DH // 2), :]
            ev, od = _interleave(a, b)
            r0 = dp * 32
            wo_p[r0:r0 + 16, c * 128:(c + 1) * 128] = ev
            wo_p[r0 + 16:r0 + 32, c * 128:(c + 1) * 128] = od
            outs.append((ev, od))
        return outs

    wait(stage_cps[0], "s0")

    def tiles8(v):
        return [jnp.broadcast_to(v[:, j * 128:(j + 1) * 128], (8, 128)) for j in range(LT)]

    wr = gw = zvec = z16 = None

    def load_vectors():
        nonlocal wr, gw, zvec, z16
        wr = tiles8(wr_vm[...].astype(f32)[None, :])
        gw = tiles8(gw_vm[...].astype(f32)[None, :])
        zero = jax.lax.shift_right_logical(
            jnp.max(jax.lax.shift_right_logical(pltpu.bitcast(wr[0], jnp.int32), 16)), 16)
        zvec = pltpu.bitcast(jnp.full((8, 128), zero, jnp.int32), u32)
        z16 = pl.multiple_of(zero * 16, 16)

    def bits(v):
        return v if v.dtype == u32 else pltpu.bitcast(v, u32)

    def token(deps):
        u = None
        for d in deps:
            d = bits(d)
            for r in range(0, d.shape[0], 8):
                part = d if d.shape[0] == 8 else d[r:r + 8]
                u = part if u is None else u | part
        return u & zvec

    def tied(v, deps):
        if not deps:
            return v
        w = bits(v) | token(deps)
        return w if v.dtype == u32 else pltpu.bitcast(w, v.dtype)

    def load_tiles(ref, g0, g1, c0, c1, deps):
        lanes = slice(c0 * 128, c1 * 128)
        rows = sorted({g * 64 + 8 * deps[(g, c)][0] for g in range(g0, g1)
                       for c in range(c0, c1) if (g, c) in deps})
        parts, prev = [], g0 * 64
        for r in rows:
            if r > prev:
                parts.append(ref[prev:r, lanes])
            cols = []
            for c in range(c0, c1):
                pos, vals = deps.get((r // 64, c), (None, None))
                cols.append(tied(ref[r:r + 8, c * 128:(c + 1) * 128],
                                 vals if pos == (r % 64) // 8 else None))
            parts.append(cols[0] if len(cols) == 1 else jnp.concatenate(cols, axis=1))
            prev = r + 8
        if prev < g1 * 64:
            parts.append(ref[prev:g1 * 64, lanes])
        w = parts[0] if len(parts) == 1 else jnp.concatenate(parts, axis=0)
        return pltpu.bitcast(w, bf16)

    def unit_a(s0, xv, n0, n1, k0, k1, deps):
        w = load_tiles(wp, n0, n1, k0, k1, deps)
        y = jax.lax.dot_general(xv, w, _NT, preferred_element_type=f32)
        outs = []
        for j in range(n0, n1):
            blk = y[:, (j - n0) * 128:(j - n0 + 1) * 128]
            outs.append(blk)
            if k0 > 0:
                blk = blk + qkv[j, HALO + s0:HALO + s0 + C, :]
            qkv[j, HALO + s0:HALO + s0 + C, :] = blk
        return outs

    def unit_c(r0, n, moe, deps):
        o = pltpu.bitcast(obuf[r0 // 2:(r0 + n) // 2, :], bf16)
        w = load_tiles(wo_p, 0, LT, 0, LT, deps)
        a = jnp.dot(o, w, preferred_element_type=f32)
        g = g_vm[r0:r0 + n, :]
        if moe is not None:
            idx, delta = moe
            row = jax.lax.broadcasted_iota(jnp.int32, (n, 128), 0) + r0
            coef = jnp.where(row == idx, 1.0 - g, 0.0)
        fences = []
        for j in range(LT):
            sl = slice(j * 128, (j + 1) * 128)
            x = x_vm[j, r0:r0 + n, :].astype(f32)
            res = x + g * (a[:, sl] - x)
            if moe is not None:
                res = res + coef * delta[j]
            out_vm[r0:r0 + n, sl] = res.astype(bf16)
            fences.append(pltpu.bitcast(out_vm[pl.ds(z16, 16), 0:128], u32))
        return [a[:, j * 128:(j + 1) * 128] for j in range(LT)], fences

    def attn_block(s0, rel):
        r0 = HALO + s0
        cq = tied(jnp.full((8, 128), CQ, f32), rel)
        q = qkv[0:LT, r0:r0 + R, :].reshape(LT * R // 8, 8, 128) * cq[None]
        q = q.reshape(LT, R, 128)
        ss = []
        for w in range(NW):
            rw = r0 - DIL * w
            s = jnp.sum(q * qkv[LT:2 * LT, rw:rw + R, :], axis=0)
            if cfg["rot2"]:
                ss.append(s + pltpu.roll(s, 64, 1))
            else:
                ss.append((s + pltpu.roll(s, 32, 1))
                          + (pltpu.roll(s, 64, 1) + pltpu.roll(s, 96, 1)))
        ls = []
        for w in range(NW):
            l = ss[w]
            if cfg["rot2"]:
                l = l + pltpu.roll(l, 32, 1)
            if s0 < DIL * w:
                row = jax.lax.broadcasted_iota(jnp.int32, (R, 128), 0) + s0
                l = jnp.where(row >= DIL * w, l, NEG)
            ls.append(l)
        m = ls[0]
        for w in range(1, NW):
            m = jnp.maximum(m, ls[w])
        ps = [jnp.exp2(l - m) for l in ls]
        den = ps[0]
        for w in range(1, NW):
            den = den + ps[w]
        inv = pl.reciprocal(den, approx=True)
        for _ in range(cfg["newton"]):
            inv = inv + inv * (1.0 - den * inv)
        o = ps[0][None] * qkv[2 * LT:3 * LT, r0:r0 + R, :]
        for w in range(1, NW):
            rw = r0 - DIL * w
            o = o + ps[w][None] * qkv[2 * LT:3 * LT, rw:rw + R, :]
        o = o * inv[None]
        outs = []
        for j in range(LT):
            ob = pltpu.bitcast(o[j].astype(bf16), u32)
            obuf[s0 // 2:(s0 + R) // 2, j * 128:(j + 1) * 128] = ob
            outs.append(o[j] if cfg["tie_f32"] else ob)
        return m, inv, outs

    def rowdot(mat, vec, stag=None):
        n = mat[0].shape[0]
        acc = None
        for j in range(LT):
            p = mat[j].reshape(n // 8, 8, 128) * vec[j][None]
            acc = p if acc is None else acc + p
        if stag is not None:
            acc = acc.reshape(len(stag), n // 8 // len(stag), 8, 128)
            acc = pltpu.bitcast(pltpu.bitcast(acc, u32) | stag[:, None], f32)
        acc = acc.reshape(n, 128)
        return jnp.broadcast_to(jnp.sum(acc, axis=-1, keepdims=True), (n, 128))

    def pre_block(b, racc, rel, stag):
        lane = jax.lax.broadcasted_iota(jnp.int32, (PR, 128), 1)
        xf = [x_vm[j, b * PR:(b + 1) * PR, :].astype(f32) for j in range(LT)]
        if stag is not None:
            rel = None
        g_vm[b * PR:(b + 1) * PR, :] = _sigmoid(rowdot(xf, [tied(v, rel) for v in gw], stag))
        return jnp.where(lane == b, rowdot(xf, [tied(v, rel) for v in wr], stag), racc)

    def ffn_block(b, xsel, yacc, rel, stag):
        f0 = b * FB
        xr = [tied(v, rel if stag is None else None) for v in xsel]
        wg = wg_vm[f0:f0 + FB, :].astype(f32)
        wu = wu_vm[f0:f0 + FB, :].astype(f32)
        gt = rowdot([wg[:, j * 128:(j + 1) * 128] for j in range(LT)], xr, stag)
        up = rowdot([wu[:, j * 128:(j + 1) * 128] for j in range(LT)], xr, stag)
        h = gt * _sigmoid(gt) * up
        new = []
        for j in range(LT):
            p = wd_vm[f0:f0 + FB, j * 128:(j + 1) * 128].astype(f32) * h
            new.append(yacc[j] + jnp.sum(p.reshape(FB // 8, 8, 128), axis=0))
        return new

    def fence_g():
        return g_vm[pl.ds(z16, 8), :]

    nfb = F // FB
    npb = S // PR
    st = dict(
        now=0.0, busy=1e9, last_side=False,
        a_row=0, b_row=0, c_row=0, p=0, f=0, w=0,
        x_avail=0, wo_avail=False, until=None,
        qkv_ready=[(0, -1e9)],
        b_ready=[(0, -1e9)],
        slot_out=[],
        due=[],
        ffn_from=None, last_c=0, main=False, c_spans=[],
        racc=jnp.full((PR, 128), -jnp.inf, f32),
        xsel=None, yacc=None, moe=None,
    )

    def avail(lst, t):
        return max(r for r, u in lst if u <= t)

    def barrier(copies, until=None, items=True):
        for cp, name in copies:
            wait(cp, name)
        st["slot_out"] = []
        st["due"] = []
        st["busy"] = st["now"] + cfg["first"] if items else 1e9
        st["until"] = until
        st["nxt"] = st["now"] + cfg["phase"] / LT
        st["pass"] = 0

    def place_item(t):
        if t < st["busy"]:
            return
        if st["until"] is not None and t >= st["until"] - cfg["quiet"]:
            return
        rels = [v for (u, v) in st["slot_out"] if u <= t - cfg["gap"]]
        rel = [v[0:8] for v in rels[-1:]]
        stag = None
        if rels and cfg["stagger"]:
            v = rels[-1]
            ng = cfg["stagger"]
            stag = lambda: (pltpu.bitcast(v.reshape(ng, v.shape[0] // 8 // ng, 8, 128)[:, 0], u32)
                            & zvec[None])
        due = st["due"]
        can_p = st["p"] * PR < st["x_avail"]
        can_w = st["wo_avail"] and st["w"] < LT
        can_f = st["ffn_from"] is not None and t >= st["ffn_from"] and st["f"] < nfb
        p_urgent = st["p"] * PR < min(st["x_avail"], st["b_row"] + cfg["p_ahead"])
        b_urgent = st["a_row"] - st["b_row"] > cfg["b_behind"] and not can_w
        if cfg["c_calm"] is not None:
            u = t - cfg["gap"]
            if any(c0 + cfg["c_calm"][0] <= u <= c1 + cfg["c_calm"][1] for c0, c1 in st["c_spans"]):
                b_urgent = True
        take_b = (st["b_row"] + R <= avail(st["qkv_ready"], t - cfg["b_slack"])
                  and not p_urgent
                  and (b_urgent or st["last_side"] or not (can_p or can_w or can_f)))
        st["last_side"] = not take_b
        if take_b:
            m, inv, obs = attn_block(st["b_row"], rel)
            if cfg["sm_off"] is not None:
                due.append((t + cfg["sm_off"][0], m))
                due.append((t + cfg["sm_off"][1], inv))
            for j, ob in enumerate(obs):
                due.append((t + cfg["pv_off"][j], ob))
            st["b_row"] += R
            st["b_ready"].append((st["b_row"], t + cfg["pv_off"][-1] + 0.2))
            width = cfg["w_b"] if st["a_row"] < S else cfg["w_b_tail"]
        elif can_w and not p_urgent:
            for dp, (ev, od) in enumerate(permute_wo(st["w"])):
                due.append((t + dp * cfg["s_w"], ev))
                due.append((t + dp * cfg["s_w"], od))
            st["w"] += 1
            width = cfg["w_w"] if st["main"] else cfg["w_p_early"]
        elif can_p:
            st["racc"] = pre_block(st["p"], st["racc"], rel, stag and stag())
            for u in range(PR // 8):
                due.append((t + u * 0.1, st["racc"][u * 8:(u + 1) * 8]))
            due.append((t + 0.8, fence_g()))
            st["p"] += 1
            width = cfg["w_p"] if st["main"] else cfg["w_p_early"]
        elif can_f:
            st["yacc"] = ffn_block(st["f"], st["xsel"], st["yacc"], rel, stag and stag())
            for j in range(LT):
                due.append((t + cfg["f_off"][j], st["yacc"][j]))
            st["f"] += 1
            width = cfg["w_f"]
        else:
            st["last_side"] = False
            return
        st["busy"] = max(st["busy"], t - cfg["grid"] / LT + 0.01) + width - 1e-6

    def plan_unit(passes, dur):
        deps = {}
        t0 = st["now"]
        for i, tile in enumerate(passes):
            t = t0 + i * dur
            if t >= st["nxt"] - 1e-6:
                place_item(t)
                st["nxt"] = t + cfg["grid"] * dur
            vals = [v for (u, v) in st["due"] if u <= t + 1e-6]
            st["due"] = [(u, v) for (u, v) in st["due"] if u > t + 1e-6]
            if vals:
                deps[tile] = (cfg["pos"][st["pass"] % 4], vals)
            st["pass"] += 1
        st["now"] = t0 + len(passes) * dur
        return deps

    def run_a(s0, xv, n0, n1, k0, k1):
        t0 = st["now"]
        deps = plan_unit([(n, kk) for n in range(n0, n1) for kk in range(k0, k1)], 1.0 / LT)
        outs = unit_a(s0, xv, n0, n1, k0, k1, deps)
        step = (k1 - k0) / LT
        st["slot_out"] += [(t0 + j * step, v) for j, v in enumerate(outs)]

    kdone = [[0] * 3 for _ in range(S // C)]
    xhave = [0] * LT
    whave = set()

    def part(b, k1, t0=0, t1=3, hook=None):
        xvs = {}
        for t in range(t0, t1):
            k0 = kdone[b][t]
            if k0 >= k1:
                continue
            assert all(xhave[j] > b and (j, t) in whave for j in range(k0, k1)), (b, t, k1)
            if k0 not in xvs:
                xvs[k0] = x_lhs(b * C, k0, k1)
            xv = xvs[k0]
            grp = max(1, cfg["a_passes"] // (k1 - k0))
            for n0 in range(t * LT, (t + 1) * LT, grp):
                if hook is not None:
                    hook()
                run_a(b * C, xv, n0, min((t + 1) * LT, n0 + grp), k0, k1)
            kdone[b][t] = k1
        if min(kdone[b]) == LT:
            assert st["a_row"] == b * C
            st["a_row"] += C
            st["qkv_ready"].append((st["a_row"], st["now"]))

    def enter_stage(n, **kw):
        barrier([(stage_cps[n], "s%d" % n)] if n else [], **kw)
        for pc in stages[n][0]:
            if pc[0] == "x":
                assert xhave[pc[1]] == pc[2]
                xhave[pc[1]] = pc[3]
            elif pc[0] == "w":
                permute_w(*pc[1:])
                whave.update((pc[1], t) for t in range(pc[2], pc[3]))
            elif pc[0] == "wo":
                st["wo_avail"] = True
            elif pc[0] == "vec":
                load_vectors()
        st["x_avail"] = min(xhave) * C
        if any(pc[0] == "w" for pc in stages[n][0]):
            st["busy"] += cfg["first_perm"] if st["main"] else cfg["first_early"]
        for pt in stages[n][1]:
            part(*pt)

    n_main = len(stages) - 2
    for n in range(n_main):
        k_sim = [list(k) for k in kdone]
        length = 0
        for pt in stages[n][1]:
            b, k1, t0, t1 = (tuple(pt) + (0, 3))[:4]
            for t in range(t0, t1):
                length += max(0, k1 - k_sim[b][t])
                k_sim[b][t] = max(k1, k_sim[b][t])
        enter_stage(n, items=(n == n_main - 1), until=st["now"] + length)
    t_main = st["now"]
    st["main"] = True
    enter_stage(n_main, until=t_main + cfg["late_t"])

    idx = r_sel = tile0 = None
    out_copies = []
    out_done = 0

    def moe_steps():
        nonlocal idx, r_sel, tile0, out_done
        if st["p"] == npb and idx is None:
            rb = st["racc"].astype(bf16).astype(f32)
            rb = jnp.where(rb != rb, -jnp.inf, rb)
            rmax = jnp.max(rb)
            rowid = (jax.lax.broadcasted_iota(jnp.int32, (PR, 128), 1) * PR
                     + jax.lax.broadcasted_iota(jnp.int32, (PR, 128), 0))
            idx = jnp.min(jnp.where((rowid < S) & (rb == rmax), rowid, S - 1))
            tile0 = pl.multiple_of((idx // 16) * 16, 16)
            r_sel = _sigmoid(jnp.full((1, 128), rmax, f32))
            row16 = jax.lax.broadcasted_iota(jnp.int32, (16, 128), 0) + tile0
            st["xsel"] = [
                jnp.broadcast_to(jnp.sum(
                    jnp.where(row16 == idx,
                              x_vm[j, pl.ds(tile0, 16), :].astype(f32), 0.0),
                    axis=0, keepdims=True), (8, 128)) for j in range(LT)]
            st["yacc"] = [jnp.zeros((8, 128), f32) for _ in range(LT)]
            st["ffn_from"] = st["now"] + cfg["router_gap"]
        elif st["f"] == nfb and st["moe"] is None:
            delta = [jnp.sum(y, axis=0, keepdims=True) * r_sel for y in st["yacc"]]
            st["moe"] = (idx, delta)
            fix_rows = st["c_row"]
            t0 = pl.multiple_of(jnp.minimum(tile0, fix_rows - 16), 16)
            row = jax.lax.broadcasted_iota(jnp.int32, (16, 128), 0) + t0
            coef = jnp.where(row == idx, 1.0 - g_vm[pl.ds(t0, 16), :], 0.0)
            cur = out_vm[pl.ds(t0, 16), :].astype(f32)
            upd = jnp.concatenate([coef * delta[j] for j in range(LT)], axis=1)
            out_vm[pl.ds(t0, 16), :] = (cur + upd).astype(bf16)
            cp = out_copy(0, fix_rows)
            cp[0].start()
            out_copies.append(cp)
            out_done = fix_rows

    def late_barrier():
        if (st["x_avail"] < S and st["now"] >= t_main + cfg["late_t"] - 1e-6
                and (st["pass"] % 4 == 0 or st["now"] >= t_main + cfg["late_t"] + 4)):
            if cfg.get("verbose"):
                print("late barrier at", st["now"] - t_main, "pass", st["pass"])
            enter_stage(n_main + 1)

    while st["c_row"] < S:
        late_barrier()
        a_row, c_row = st["a_row"], st["c_row"]
        cc = cfg["CC"] if c_row < S - cfg["tail_rows"] else cfg["tail_cc"]
        c_ok = (avail(st["b_ready"], st["now"] - cfg["c_slack"]) >= c_row + cc
                and st["p"] * PR >= c_row + cc and st["w"] == LT)
        units = []
        if a_row < S and (not c_ok or a_row - c_row < cfg["c_lag"] or st["last_c"] >= cfg["c_run"]):
            units = ["a"]
            st["last_c"] = 0
        elif c_ok:
            units = ["c"]
            st["last_c"] += 1
        else:
            place_item(st["now"])
            st["due"] = []
            st["now"] += 1.0
        for kind in units:
            if kind == "a":
                part(a_row // C, LT, hook=lambda: (late_barrier(), moe_steps()))
            else:
                t0 = st["now"]
                dur = cc / C
                st["c_spans"].append((t0, t0 + LT * dur))
                deps = plan_unit([(kk, n) for n in range(LT) for kk in range(LT)], dur / LT)
                outs, fences = unit_c(c_row, cc, st["moe"], deps)
                st["slot_out"] += [(t0 + j * dur, v) for j, v in enumerate(outs)]
                st["c_row"] += cc
                for j in range(cfg["fence_from"], LT):
                    st["due"].append((t0 + (j + 1) * dur + cfg["fence_lag"], fences[j]))
                st["busy"] = max(st["busy"], st["now"] - 1) + cfg["w_c"] * dur
                if st["moe"] is not None and (st["c_row"] in cfg["out_splits"]
                                              or st["c_row"] == S):
                    cp = out_copy(out_done, st["c_row"])
                    cp[0].start()
                    out_copies.append(cp)
                    out_done = st["c_row"]
            moe_steps()
        if cfg.get("verbose"):
            print(round(st["now"] - t_main, 1),
                  {k: st[k] for k in ("a_row", "b_row", "c_row", "p", "f", "w")})

    assert out_done == S
    for n, cp in enumerate(out_copies):
        wait(cp, "o%d" % n)


def _kernel_once(*refs, cfg):
    pl.when(pl.program_id(0) == cfg["step"])(lambda: _kernel(*refs, cfg=cfg))


def _build(cfg):
    bf16 = jnp.bfloat16
    f32 = jnp.float32
    u32 = jnp.uint32
    hbm_spec = pl.BlockSpec(memory_space=pltpu.MemorySpace.HBM)
    return pl.pallas_call(
        functools.partial(_kernel_once, cfg=cfg),
        grid=(2,),
        out_shape=jax.ShapeDtypeStruct((1, S, D), bf16),
        in_specs=[hbm_spec] * 8,
        out_specs=hbm_spec,
        scratch_shapes=[
            pltpu.VMEM((LT, S, 128), bf16),
            pltpu.VMEM((D, 3 * D), bf16),
            pltpu.VMEM((LT, 3, D // 2 + 16, 128), u32),
            pltpu.VMEM((3 * D // 2, D), u32),
            pltpu.VMEM((LT, D, 128), bf16),
            pltpu.VMEM((LT, D // 2 + 16, 128), u32),
            pltpu.VMEM((D // 2, D), u32),
            pltpu.VMEM((D,), bf16),
            pltpu.VMEM((D,), bf16),
            pltpu.VMEM((F, D), bf16),
            pltpu.VMEM((F, D), bf16),
            pltpu.VMEM((F, D), bf16),
            pltpu.VMEM((3 * LT, HALO + S, 128), f32),
            pltpu.VMEM((S // 2, D), u32),
            pltpu.VMEM((S, D), bf16),
            pltpu.VMEM((S, 128), f32),
            pltpu.SemaphoreType.DMA((40 + len(cfg["out_splits"]) + 2,)),
        ],
        compiler_params=pltpu.CompilerParams(
            dimension_semantics=("arbitrary",),
            vmem_limit_bytes=100 * 1024 * 1024,
            disable_bounds_checks=True,
            disable_semaphore_checks=True),
    )


def _call(cfg, A_x, A_wqkv, A_wo, B_w_r, B_w_gate, B_w_up, B_w_down, gate_w):
    return _build(cfg)(A_x, A_wqkv, A_wo, B_w_r, B_w_gate.T, B_w_up.T, B_w_down, gate_w)


@jax.jit
def pallas_gated_mix__sliding_local_dilated__moe_arch_mod__prompt_kernel(
    A_x: jax.Array,
    A_wqkv: jax.Array,
    A_wo: jax.Array,
    B_x: jax.Array,
    B_w_r: jax.Array,
    B_w_gate: jax.Array,
    B_w_up: jax.Array,
    B_w_down: jax.Array,
    gate_w: jax.Array,
):
    del B_x
    return _call(CFG, A_x, A_wqkv, A_wo, B_w_r, B_w_gate, B_w_up, B_w_down, gate_w)
```

```python
import functools

import jax
import jax.numpy as jnp
import jax.experimental.pallas as pl
import jax.experimental.pallas.tpu as pltpu

S = 2048
D = 640
H = 32
DH = 20
NW = 8
DIL = 2
F = 1728
LT = D // 128
HALO = 16
LOG2E = 1.4426950408889634
CQ = (DH ** -0.5) * LOG2E
NEG = -1e9 * LOG2E
C = 128
R = 16
PR = 64
FB = 64

_NT = (((1,), (1,)), ((), ()))

CFG = dict(
    CC=128,
    tail_rows=256,
    tail_cc=64,
    a_passes=5,
    z=(6, 10, 2, 5, 6, 9),
    late_t=92,
    w_b=1.6, w_p=0.8, w_f=0.8, w_w=0.8,
    pv_off=(0.0, 0.2, 0.6, 0.8, 1.2),
    f_off=(0.0, 0.2, 0.6, 0.8, 1.2),
    s_w=0.1,
    gap_r=6, rel_row=6,
    stagger=8,
    pos=(7, 5, 3, 0),
    first=2.4,
    first_perm=9.6,
    quiet=1,
    c_lag=512,
    c_slack=2.0,
    b_slack=2.5,
    b_behind=300,
    p_ahead=64,
    fence_lag=3,
    router_gap=6,
    out_splits=(1664, 1792, 1920, 1984),
    last_tiles=(1, 3, 4),
)


def _stages(cfg):
    NB = S // C
    xs = lambda js, b0, b1: [("x", j, b0, b1) for j in js]
    w = lambda kk, t0=0, t1=3: ("w", kk, t0, t1)
    na, m0, h, m1, mx, xc = cfg["z"]
    return [
        ([w(0, 0, 1)], []),
        (xs([0], 0, na), [(b, 1, 0, 1) for b in range(na)]),
        ([w(0, 1, 3), ("vec",)] + xs([0], na, m0),
         [(b, 1, 0, 1) for b in range(na, m0)] + [(b, 1) for b in range(m0 - h)]),
        ([w(1), w(2)] + xs([1, 2, 3, 4], 0, mx),
         [(b, 1) for b in range(m0 - h, m0)] + [(0, 2), (0, 3)]
         + [(b, 3) for b in range(1, m1 - 1)]),
        ([w(3), w(4)] + (xs([0], m0, xc) if xc > m0 else [])
         + xs([1, 2, 3, 4], mx, xc) + [("wo",)],
         [(m1 - 1, 3), (0, 4)]),
        (xs([0], max(m0, xc), NB) + xs([1, 2, 3, 4], xc, NB) + [("ffn",)], []),
    ]


def _sigmoid(z):
    return 0.5 * jnp.tanh(0.5 * z) + 0.5


def _interleave(a, b):
    ev = (a & jnp.uint32(0xFFFF)) | (b << 16)
    od = (a >> 16) | (b & jnp.uint32(0xFFFF0000))
    return ev, od


def _kernel(x_hbm, w_hbm, wo_hbm, wr_hbm, wg_hbm, wu_hbm, wd_hbm, gw_hbm,
            out_hbm,
            x_vm, w_raw, tscr, wp, wo_raw, wo_u32, wo_p, wr_vm, gw_vm,
            wg_vm, wu_vm, wd_vm, qkv, obuf, out_vm, g_vm,
            sems, *, cfg):
    f32 = jnp.float32
    bf16 = jnp.bfloat16
    u32 = jnp.uint32

    nsem = [0]

    def copy(src, dst):
        nsem[0] += 1
        return pltpu.make_async_copy(src, dst, sems.at[nsem[0] - 1])

    def piece(pc):
        if pc[0] == "x":
            _, j, b0, b1 = pc
            rows = pl.ds(b0 * C, (b1 - b0) * C)
            return [copy(x_hbm.at[0, rows, pl.ds(j * 128, 128)], x_vm.at[j, rows, :])]
        if pc[0] == "w":
            _, kk, t0, t1 = pc
            rows, cols = pl.ds(kk * 128, 128), pl.ds(t0 * D, (t1 - t0) * D)
            return [copy(w_hbm.at[rows, cols], w_raw.at[rows, cols])]
        if pc[0] == "wo":
            return [copy(wo_hbm.at[:, pl.ds(j * 128, 128)], wo_raw.at[j])
                    for j in range(LT)]
        if pc[0] == "vec":
            return [copy(wr_hbm, wr_vm), copy(gw_hbm, gw_vm)]
        assert pc[0] == "ffn"
        return [copy(wg_hbm, wg_vm), copy(wu_hbm, wu_vm), copy(wd_hbm, wd_vm)]

    stages = _stages(cfg)
    stage_cps = [[cp for pc in sg[0] for cp in piece(pc)] for sg in stages]

    def out_copy(r0, r1):
        return [copy(out_vm.at[pl.ds(r0, r1 - r0), :], out_hbm.at[0, pl.ds(r0, r1 - r0), :])]

    def x_lhs(s0, k0, k1):
        cols = [pltpu.bitcast(x_vm[j, s0:s0 + C, :], u32) for j in range(k0, k1)]
        return pltpu.bitcast(cols[0] if len(cols) == 1 else jnp.concatenate(cols, axis=1), bf16)

    def wait(cps, name):
        if cfg.get("scopes"):
            with jax.named_scope("wait_" + name):
                for cp in cps:
                    cp.wait()
        else:
            for cp in cps:
                cp.wait()

    for cps in stage_cps:
        for cp in cps:
            cp.start()

    qkv[LT:3 * LT, 0:HALO, :] = jnp.zeros((2 * LT, HALO, 128), f32)

    def permute_w(kk, t0, t1):
        for t in range(t0, t1):
            for c in range(LT):
                tile = w_raw[kk * 128:(kk + 1) * 128,
                             t * D + c * 128:t * D + (c + 1) * 128]
                tscr[kk, t, c * 64:(c + 1) * 64, :] = pltpu.bitcast(tile.T, u32)
        for t in range(t0, t1):
            for dp in range(DH // 2):
                a = tscr[kk, t, pl.ds(dp, 16, stride=DH // 2), :]
                b = tscr[kk, t, pl.ds(160 + dp, 16, stride=DH // 2), :]
                ev, od = _interleave(a, b)
                r0 = (t * D + 2 * dp * 32) // 2
                wp[r0:r0 + 16, kk * 128:(kk + 1) * 128] = ev
                wp[r0 + 16:r0 + 32, kk * 128:(kk + 1) * 128] = od

    def permute_wo(c):
        wo_u32[c, 0:D // 2, :] = pltpu.bitcast(wo_raw[c], u32)
        outs = []
        for dp in range(DH // 2):
            a = wo_u32[c, pl.ds(dp, 16, stride=DH // 2), :]
            b = wo_u32[c, pl.ds(160 + dp, 16, stride=DH // 2), :]
            ev, od = _interleave(a, b)
            r0 = dp * 32
            wo_p[r0:r0 + 16, c * 128:(c + 1) * 128] = ev
            wo_p[r0 + 16:r0 + 32, c * 128:(c + 1) * 128] = od
            outs.append((ev, od))
        return outs

    wait(stage_cps[0], "s0")

    def tiles8(v):
        return [jnp.broadcast_to(v[:, j * 128:(j + 1) * 128], (8, 128)) for j in range(LT)]

    wr = gw = zvec = z16 = None

    def load_vectors():
        nonlocal wr, gw, zvec, z16
        wr = tiles8(wr_vm[...].astype(f32)[None, :])
        gw = tiles8(gw_vm[...].astype(f32)[None, :])
        zero = jax.lax.shift_right_logical(
            jnp.max(jax.lax.shift_right_logical(pltpu.bitcast(wr[0], jnp.int32), 16)), 16)
        zvec = pltpu.bitcast(jnp.full((8, 128), zero, jnp.int32), u32)
        z16 = pl.multiple_of(zero * 16, 16)

    def bits(v):
        return v if v.dtype == u32 else pltpu.bitcast(v, u32)

    def token(deps):
        u = None
        for d in deps:
            d = bits(d)
            for r in range(0, d.shape[0], 8):
                part = d if d.shape[0] == 8 else d[r:r + 8]
                u = part if u is None else u | part
        return u & zvec

    def tied(v, deps):
        if not deps:
            return v
        w = bits(v) | token(deps)
        return w if v.dtype == u32 else pltpu.bitcast(w, v.dtype)

    def load_tiles(ref, g0, g1, c0, c1, deps):
        lanes = slice(c0 * 128, c1 * 128)
        rows = sorted({g * 64 + 8 * deps[(g, c)][0] for g in range(g0, g1)
                       for c in range(c0, c1) if (g, c) in deps})
        parts, prev = [], g0 * 64
        for r in rows:
            if r > prev:
                parts.append(ref[prev:r, lanes])
            cols = []
            for c in range(c0, c1):
                pos, vals = deps.get((r // 64, c), (None, None))
                cols.append(tied(ref[r:r + 8, c * 128:(c + 1) * 128],
                                 vals if pos == (r % 64) // 8 else None))
            parts.append(cols[0] if len(cols) == 1 else jnp.concatenate(cols, axis=1))
            prev = r + 8
        if prev < g1 * 64:
            parts.append(ref[prev:g1 * 64, lanes])
        w = parts[0] if len(parts) == 1 else jnp.concatenate(parts, axis=0)
        return pltpu.bitcast(w, bf16)

    def unit_a(s0, xv, n0, n1, k0, k1, deps):
        w = load_tiles(wp, n0, n1, k0, k1, deps)
        y = jax.lax.dot_general(xv, w, _NT, preferred_element_type=f32)
        outs = []
        for j in range(n0, n1):
            blk = y[:, (j - n0) * 128:(j - n0 + 1) * 128]
            outs.append(blk)
            if k0 > 0:
                blk = blk + qkv[j, HALO + s0:HALO + s0 + C, :]
            qkv[j, HALO + s0:HALO + s0 + C, :] = blk
        return outs

    def unit_c(r0, n, moe, deps, per_tile_out=None):
        o = pltpu.bitcast(obuf[r0 // 2:(r0 + n) // 2, :], bf16)
        w = load_tiles(wo_p, 0, LT, 0, LT, deps)
        a = jnp.dot(o, w, preferred_element_type=f32)
        g = g_vm[r0:r0 + n, :]
        if moe is not None:
            idx, delta = moe
            hit = jax.lax.broadcasted_iota(jnp.int32, (n, 128), 0) + r0 == idx
        for j in range(LT):
            sl = slice(j * 128, (j + 1) * 128)
            x = x_vm[j, r0:r0 + n, :].astype(f32)
            if moe is not None:
                x = x + jnp.where(hit, delta[j], 0.0)
            res = x + g * (a[:, sl] - x)
            out_vm[r0:r0 + n, sl] = res.astype(bf16)
            if per_tile_out is not None and j in cfg["last_tiles"]:
                j0 = ([-1] + list(cfg["last_tiles"]))[cfg["last_tiles"].index(j)] + 1
                cols = pl.ds(j0 * 128, (j + 1 - j0) * 128)
                cp = copy(out_vm.at[pl.ds(r0, n), cols], out_hbm.at[0, pl.ds(r0, n), cols])
                cp.start()
                per_tile_out.append([cp])
        fence = pltpu.bitcast(out_vm[pl.ds(z16, 16), 0:128], u32)
        return [a[:, j * 128:(j + 1) * 128] for j in range(LT)], fence

    def attn_block(s0, rel):
        r0 = HALO + s0
        cq = tied(jnp.full((8, 128), CQ, f32), rel)
        q = qkv[0:LT, r0:r0 + R, :].reshape(LT * R // 8, 8, 128) * cq[None]
        q = q.reshape(LT, R, 128)
        ls = []
        for w in range(NW):
            rw = r0 - DIL * w
            s = jnp.sum(q * qkv[LT:2 * LT, rw:rw + R, :], axis=0)
            l = (s + pltpu.roll(s, 32, 1)) + (pltpu.roll(s, 64, 1) + pltpu.roll(s, 96, 1))
            if s0 < DIL * w:
                row = jax.lax.broadcasted_iota(jnp.int32, (R, 128), 0) + s0
                l = jnp.where(row >= DIL * w, l, NEG)
            ls.append(l)
        m = ls[0]
        for w in range(1, NW):
            m = jnp.maximum(m, ls[w])
        ps = [jnp.exp2(l - m) for l in ls]
        den = ps[0]
        for w in range(1, NW):
            den = den + ps[w]
        inv = pl.reciprocal(den, approx=True)
        inv = inv + inv * (1.0 - den * inv)
        o = ps[0][None] * qkv[2 * LT:3 * LT, r0:r0 + R, :]
        for w in range(1, NW):
            rw = r0 - DIL * w
            o = o + ps[w][None] * qkv[2 * LT:3 * LT, rw:rw + R, :]
        o = o * inv[None]
        outs = []
        for j in range(LT):
            oj = o[j]
            obuf[s0 // 2:(s0 + R) // 2, j * 128:(j + 1) * 128] = pltpu.bitcast(
                oj.astype(bf16), u32)
            outs.append(oj)
        return m, inv, outs

    def rowdot(mat, vec, stag=None):
        n = mat[0].shape[0]
        acc = None
        for j in range(LT):
            p = mat[j].reshape(n // 8, 8, 128) * vec[j][None]
            acc = p if acc is None else acc + p
        if stag is not None:
            acc = acc.reshape(len(stag), n // 8 // len(stag), 8, 128)
            acc = pltpu.bitcast(pltpu.bitcast(acc, u32) | stag[:, None], f32)
        acc = acc.reshape(n, 128)
        return jnp.broadcast_to(jnp.sum(acc, axis=-1, keepdims=True), (n, 128))

    def pre_block(b, racc, stag):
        lane = jax.lax.broadcasted_iota(jnp.int32, (PR, 128), 1)
        xf = [x_vm[j, b * PR:(b + 1) * PR, :].astype(f32) for j in range(LT)]
        g_vm[b * PR:(b + 1) * PR, :] = _sigmoid(rowdot(xf, gw, stag))
        return jnp.where(lane == b, rowdot(xf, wr, stag), racc)

    def ffn_block(b, xsel, yacc, stag):
        f0 = b * FB
        wg = wg_vm[f0:f0 + FB, :].astype(f32)
        wu = wu_vm[f0:f0 + FB, :].astype(f32)
        gt = rowdot([wg[:, j * 128:(j + 1) * 128] for j in range(LT)], xsel, stag)
        up = rowdot([wu[:, j * 128:(j + 1) * 128] for j in range(LT)], xsel, stag)
        h = gt * _sigmoid(gt) * up
        new = []
        for j in range(LT):
            p = wd_vm[f0:f0 + FB, j * 128:(j + 1) * 128].astype(f32) * h
            new.append(yacc[j] + jnp.sum(p.reshape(FB // 8, 8, 128), axis=0))
        return new

    def fence_g():
        return g_vm[pl.ds(z16, 8), :]

    nfb = F // FB
    npb = S // PR
    st = dict(
        now=0.0, busy=1e9, last_side=False,
        a_row=0, b_row=0, c_row=0, p=0, f=0, w=0,
        x_avail=0, wo_avail=False, until=None,
        qkv_ready=[(0, -1e9)],
        b_ready=[(0, -1e9)],
        slot_out=[],
        due=[],
        ffn_from=None, rtime=0.0,
        racc=jnp.full((PR, 128), -jnp.inf, f32),
        xsel=None, yacc=None, moe=None,
    )

    def avail(lst, t):
        return max(r for r, u in lst if u <= t)

    def barrier(copies, until=None, items=True):
        for cp, name in copies:
            wait(cp, name)
        st["slot_out"] = []
        st["due"] = []
        st["busy"] = st["now"] + cfg["first"] if items else 1e9
        st["until"] = until
        st["nxt"] = st["now"]
        st["pass"] = 0

    def place_item(t):
        if t < st["busy"]:
            return
        if st["until"] is not None and t >= st["until"] - cfg["quiet"]:
            return
        want = st["rtime"] - cfg["gap_r"]
        cand = [(rd, v) for (rd, v) in st["slot_out"] if rd <= want + 1e-6]

        def rel():
            if not cand:
                return []
            rd, v = cand[-1]
            r = min(v.shape[0] // 8 - 1, int((want - rd) * 16 + cfg["rel_row"] + 1e-6))
            return [v[8 * r:8 * r + 8]]

        def stag():
            if not cand:
                return None
            v, ng = cand[-1][1], cfg["stagger"]
            return bits(v.reshape(ng, v.shape[0] // 8 // ng, 8, 128)[:, 0]) & zvec[None]

        due = st["due"]
        can_p = st["p"] * PR < st["x_avail"]
        can_w = st["wo_avail"] and st["w"] < LT
        can_f = st["ffn_from"] is not None and t >= st["ffn_from"] and st["f"] < nfb
        p_urgent = st["p"] * PR < min(st["x_avail"], st["b_row"] + cfg["p_ahead"])
        b_urgent = st["a_row"] - st["b_row"] > cfg["b_behind"] and not can_w
        take_b = (st["b_row"] + R <= avail(st["qkv_ready"], t - cfg["b_slack"])
                  and not p_urgent
                  and (b_urgent or st["last_side"] or not (can_p or can_w or can_f)))
        st["last_side"] = not take_b
        if take_b:
            m, inv, obs = attn_block(st["b_row"], rel())
            due.append((t, m))
            due.append((t, inv))
            for j, ob in enumerate(obs):
                due.append((t + cfg["pv_off"][j], ob))
            st["b_row"] += R
            st["b_ready"].append((st["b_row"], t + cfg["pv_off"][-1] + 0.2))
            width = cfg["w_b"]
        elif can_w and not p_urgent:
            for dp, (ev, od) in enumerate(permute_wo(st["w"])):
                due.append((t + dp * cfg["s_w"], ev))
                due.append((t + dp * cfg["s_w"], od))
            st["w"] += 1
            width = cfg["w_w"]
        elif can_p:
            st["racc"] = pre_block(st["p"], st["racc"], stag())
            for u in range(PR // 8):
                due.append((t + u * 0.1, st["racc"][u * 8:(u + 1) * 8]))
            due.append((t + 0.8, fence_g()))
            st["p"] += 1
            width = cfg["w_p"]
        elif can_f:
            st["yacc"] = ffn_block(st["f"], st["xsel"], st["yacc"], stag())
            for j in range(LT):
                due.append((t + cfg["f_off"][j], st["yacc"][j]))
            st["f"] += 1
            width = cfg["w_f"]
        else:
            st["last_side"] = False
            return
        st["busy"] = max(st["busy"], t - 0.79) + width - 1e-6

    def plan_unit(passes, dur):
        deps = {}
        t0 = st["now"]
        st["pass_round"] = []
        for i, tile in enumerate(passes):
            t = t0 + i * dur
            if st["pass"] % 4 == 0:
                st["rtime"] = t / 0.8
            st["pass_round"].append(st["rtime"])
            if t >= st["nxt"] - 1e-6:
                place_item(t)
                st["nxt"] = t + 4 * dur
            vals = [v for (u, v) in st["due"] if u <= t + 1e-6]
            st["due"] = [(u, v) for (u, v) in st["due"] if u > t + 1e-6]
            if vals:
                deps[tile] = (cfg["pos"][st["pass"] % 4], vals)
            st["pass"] += 1
        st["now"] = t0 + len(passes) * dur
        return deps

    def run_a(s0, xv, n0, n1, k0, k1):
        deps = plan_unit([(n, kk) for n in range(n0, n1) for kk in range(k0, k1)], 1.0 / LT)
        outs = unit_a(s0, xv, n0, n1, k0, k1, deps)
        st["slot_out"] += [(st["pass_round"][(j + 1) * (k1 - k0) - 1], v)
                           for j, v in enumerate(outs)]

    kdone = [[0] * 3 for _ in range(S // C)]
    xhave = [0] * LT
    whave = set()

    def part(b, k1, t0=0, t1=3, hook=None):
        xvs = {}
        for t in range(t0, t1):
            k0 = kdone[b][t]
            if k0 >= k1:
                continue
            assert all(xhave[j] > b and (j, t) in whave for j in range(k0, k1)), (b, t, k1)
            if k0 not in xvs:
                xvs[k0] = x_lhs(b * C, k0, k1)
            xv = xvs[k0]
            grp = max(1, cfg["a_passes"] // (k1 - k0))
            for n0 in range(t * LT, (t + 1) * LT, grp):
                if hook is not None:
                    hook()
                run_a(b * C, xv, n0, min((t + 1) * LT, n0 + grp), k0, k1)
            kdone[b][t] = k1
        if min(kdone[b]) == LT:
            assert st["a_row"] == b * C
            st["a_row"] += C
            st["qkv_ready"].append((st["a_row"], st["now"]))

    def enter_stage(n, **kw):
        barrier([(stage_cps[n], "s%d" % n)] if n else [], **kw)
        for pc in stages[n][0]:
            if pc[0] == "x":
                assert xhave[pc[1]] == pc[2]
                xhave[pc[1]] = pc[3]
            elif pc[0] == "w":
                permute_w(*pc[1:])
                whave.update((pc[1], t) for t in range(pc[2], pc[3]))
            elif pc[0] == "wo":
                st["wo_avail"] = True
            elif pc[0] == "vec":
                load_vectors()
        st["x_avail"] = min(xhave) * C
        if any(pc[0] == "w" for pc in stages[n][0]):
            st["busy"] += cfg["first_perm"]
        for pt in stages[n][1]:
            part(*pt)

    n_main = len(stages) - 2
    for n in range(n_main):
        k_sim = [list(k) for k in kdone]
        length = 0
        for pt in stages[n][1]:
            b, k1, t0, t1 = (tuple(pt) + (0, 3))[:4]
            for t in range(t0, t1):
                length += max(0, k1 - k_sim[b][t])
                k_sim[b][t] = max(k1, k_sim[b][t])
        enter_stage(n, items=(n == n_main - 1), until=st["now"] + length)
    t_main = st["now"]
    enter_stage(n_main, until=t_main + cfg["late_t"])

    idx = r_sel = tile0 = None
    out_copies = []
    out_done = 0

    def moe_steps():
        nonlocal idx, r_sel, tile0, out_done
        if st["p"] == npb and idx is None:
            rb = st["racc"].astype(bf16).astype(f32)
            rb = jnp.where(rb != rb, -jnp.inf, rb)
            rmax = jnp.max(rb)
            rowid = (jax.lax.broadcasted_iota(jnp.int32, (PR, 128), 1) * PR
                     + jax.lax.broadcasted_iota(jnp.int32, (PR, 128), 0))
            idx = jnp.min(jnp.where((rowid < S) & (rb == rmax), rowid, S - 1))
            tile0 = pl.multiple_of((idx // 16) * 16, 16)
            r_sel = _sigmoid(jnp.full((1, 128), rmax, f32))
            row16 = jax.lax.broadcasted_iota(jnp.int32, (16, 128), 0) + tile0
            st["xsel"] = [
                jnp.broadcast_to(jnp.sum(
                    jnp.where(row16 == idx,
                              x_vm[j, pl.ds(tile0, 16), :].astype(f32), 0.0),
                    axis=0, keepdims=True), (8, 128)) for j in range(LT)]
            st["yacc"] = [jnp.zeros((8, 128), f32) for _ in range(LT)]
            st["ffn_from"] = st["now"] + cfg["router_gap"]
        elif st["f"] == nfb and st["moe"] is None:
            delta = [jnp.sum(y, axis=0, keepdims=True) * r_sel for y in st["yacc"]]
            st["moe"] = (idx, delta)
            fix_rows = st["c_row"]
            t0 = pl.multiple_of(jnp.minimum(tile0, fix_rows - 16), 16)
            row = jax.lax.broadcasted_iota(jnp.int32, (16, 128), 0) + t0
            coef = 1.0 - g_vm[pl.ds(t0, 16), :]
            cur = out_vm[pl.ds(t0, 16), :].astype(f32)
            upd = jnp.concatenate(
                [jnp.where(row == idx, coef * delta[j], 0.0) for j in range(LT)], axis=1)
            out_vm[pl.ds(t0, 16), :] = (cur + upd).astype(bf16)
            cp = out_copy(0, fix_rows)
            cp[0].start()
            out_copies.append(cp)
            out_done = fix_rows

    def late_barrier():
        if (st["x_avail"] < S and st["now"] >= t_main + cfg["late_t"] - 1e-6
                and (st["pass"] % 4 == 0 or st["now"] >= t_main + cfg["late_t"] + 4)):
            if cfg.get("verbose"):
                print("late barrier at", st["now"] - t_main, "pass", st["pass"])
            enter_stage(n_main + 1)

    while st["c_row"] < S:
        late_barrier()
        a_row, c_row = st["a_row"], st["c_row"]
        cc = cfg["CC"] if c_row < S - cfg["tail_rows"] else cfg["tail_cc"]
        c_ok = (avail(st["b_ready"], st["now"] - cfg["c_slack"]) >= c_row + cc
                and st["p"] * PR >= c_row + cc and st["w"] == LT)
        units = []
        if a_row < S and (not c_ok or a_row - c_row < cfg["c_lag"]):
            units = ["a"]
        elif c_ok:
            units = ["c"]
        else:
            place_item(st["now"])
            st["due"] = []
            st["now"] += 1.0
        for kind in units:
            if kind == "a":
                part(a_row // C, LT, hook=lambda: (late_barrier(), moe_steps()))
            else:
                dur = cc / C
                deps = plan_unit([(kk, n) for n in range(LT) for kk in range(LT)], dur / LT)
                split = cfg["last_tiles"] and c_row + cc == S and out_done == c_row
                outs, fence = unit_c(c_row, cc, st["moe"], deps,
                                      out_copies if split else None)
                if split:
                    out_done = S
                st["slot_out"] += [(st["pass_round"][(j + 1) * LT - 1], v)
                                   for j, v in enumerate(outs)]
                st["c_row"] += cc
                st["due"].append((st["now"] + cfg["fence_lag"], fence))
                st["busy"] = max(st["busy"], st["now"] - 1)
                if st["moe"] is not None and out_done < S and (
                        st["c_row"] in cfg["out_splits"] or st["c_row"] == S):
                    cp = out_copy(out_done, st["c_row"])
                    cp[0].start()
                    out_copies.append(cp)
                    out_done = st["c_row"]
            moe_steps()
        if cfg.get("verbose"):
            print(round(st["now"] - t_main, 1),
                  {k: st[k] for k in ("a_row", "b_row", "c_row", "p", "f", "w")})

    assert out_done == S
    for n, cp in enumerate(out_copies):
        wait(cp, "o%d" % n)


def _kernel_once(*refs, cfg):
    pl.when(pl.program_id(0) == 0)(lambda: _kernel(*refs, cfg=cfg))


def _build(cfg):
    bf16 = jnp.bfloat16
    f32 = jnp.float32
    u32 = jnp.uint32
    hbm_spec = pl.BlockSpec(memory_space=pltpu.MemorySpace.HBM)
    no_checks = {k: True for k in ("disable_bounds_checks", "disable_semaphore_checks")
                 if hasattr(pltpu.CompilerParams, k)}
    return pl.pallas_call(
        functools.partial(_kernel_once, cfg=cfg),
        grid=(2,),
        out_shape=jax.ShapeDtypeStruct((1, S, D), bf16),
        in_specs=[hbm_spec] * 8,
        out_specs=hbm_spec,
        scratch_shapes=[
            pltpu.VMEM((LT, S, 128), bf16),
            pltpu.VMEM((D, 3 * D), bf16),
            pltpu.VMEM((LT, 3, D // 2 + 16, 128), u32),
            pltpu.VMEM((3 * D // 2, D), u32),
            pltpu.VMEM((LT, D, 128), bf16),
            pltpu.VMEM((LT, D // 2 + 16, 128), u32),
            pltpu.VMEM((D // 2, D), u32),
            pltpu.VMEM((D,), bf16),
            pltpu.VMEM((D,), bf16),
            pltpu.VMEM((F, D), bf16),
            pltpu.VMEM((F, D), bf16),
            pltpu.VMEM((F, D), bf16),
            pltpu.VMEM((3 * LT, HALO + S, 128), f32),
            pltpu.VMEM((S // 2, D), u32),
            pltpu.VMEM((S, D), bf16),
            pltpu.VMEM((S, 128), f32),
            pltpu.SemaphoreType.DMA((48 + len(cfg["out_splits"]),)),
        ],
        compiler_params=pltpu.CompilerParams(
            dimension_semantics=("arbitrary",),
            vmem_limit_bytes=100 * 1024 * 1024,
            **no_checks),
    )


def _call(cfg, A_x, A_wqkv, A_wo, B_w_r, B_w_gate, B_w_up, B_w_down, gate_w):
    return _build(cfg)(A_x, A_wqkv, A_wo, B_w_r, B_w_gate.T, B_w_up.T, B_w_down, gate_w)


@jax.jit
def pallas_gated_mix__sliding_local_dilated__moe_arch_mod__prompt_kernel(
    A_x: jax.Array,
    A_wqkv: jax.Array,
    A_wo: jax.Array,
    B_x: jax.Array,
    B_w_r: jax.Array,
    B_w_gate: jax.Array,
    B_w_up: jax.Array,
    B_w_down: jax.Array,
    gate_w: jax.Array,
):
    del B_x
    return _call(CFG, A_x, A_wqkv, A_wo, B_w_r, B_w_gate, B_w_up, B_w_down, gate_w)
```

```python
import functools

import jax
import jax.numpy as jnp
import jax.experimental.pallas as pl
import jax.experimental.pallas.tpu as pltpu

S = 2048
D = 640
H = 32
DH = 20
NW = 8
DIL = 2
F = 1728
LT = D // 128
HALO = 16
LOG2E = 1.4426950408889634
CQ = (DH ** -0.5) * LOG2E
NEG = -1e9 * LOG2E
C = 128
R = 16
PR = 64
FB = 64

_NT = (((1,), (1,)), ((), ()))

CFG = dict(
    CC=128,
    tail_rows=256,
    tail_cc=64,
    a_passes=5,
    z=(6, 10, 2, 5, 6, 9),
    halves=((4, 0, 1), (5, 0, 1)),
    late_t=92,
    w_b=1.6, w_p=0.8, w_f=0.8, w_w=0.8,
    pv_off=(0.0, 0.2, 0.6, 0.8, 1.0),
    f_off=(0.0, 0.4, 0.6, 1.0, 1.4),
    s_w=0.1,
    gap_r=6, rel_row=6,
    stagger=8,
    pos=(7, 5, 3, 0),
    first=2.4,
    first_perm=9.6,
    quiet=1,
    c_lag=512,
    c_slack=2.0,
    b_slack=2,
    b_behind=300,
    p_ahead=64,
    fence_lag=3.4,
    router_gap=5,
    out_splits=(1664, 1792, 1920, 1984),
    last_tiles=(1, 3, 4),
)


def _stages(cfg):
    NB = S // C
    xs = lambda js, b0, b1: [("x", j, b0, b1) for j in js]
    w = lambda kk, t0=0, t1=3: ("w", kk, t0, t1)
    na, m0, h, m1, mx, xc = cfg["z"]
    return [
        ([w(0, 0, 1)], []),
        (xs([0], 0, na), [(b, 1, 0, 1) for b in range(na)]),
        ([w(0, 1, 3), ("vec",)] + xs([0], na, m0),
         [(b, 1, 0, 1) for b in range(na, m0)] + [(b, 1) for b in range(m0 - h)]),
        ([w(1), w(2)] + xs([1, 2, 3, 4], 0, mx),
         [(b, 1) for b in range(m0 - h, m0)] + [(0, 2), (0, 3)]
         + [(b, 3) for b in range(1, m1 - 1)]),
        ([w(3), w(4)] + (xs([0], m0, xc) if xc > m0 else [])
         + xs([1, 2, 3, 4], mx, xc) + [("wo",)],
         [(m1 - 1, 3), (0, 4)]),
        (xs([0], max(m0, xc), NB) + xs([1, 2, 3, 4], xc, NB) + [("ffn",)], []),
    ]


def _sigmoid(z):
    return 0.5 * jnp.tanh(0.5 * z) + 0.5


def _interleave(a, b):
    ev = (a & jnp.uint32(0xFFFF)) | (b << 16)
    od = (a >> 16) | (b & jnp.uint32(0xFFFF0000))
    return ev, od


def _kernel(x_hbm, w_hbm, wo_hbm, wr_hbm, wg_hbm, wu_hbm, wd_hbm, gw_hbm,
            out_hbm,
            x_vm, w_raw, tscr, wp, wo_raw, wo_u32, wo_p, wr_vm, gw_vm,
            wg_vm, wu_vm, wd_vm, qkv, obuf, out_vm, g_vm,
            sems, *, cfg):
    f32 = jnp.float32
    bf16 = jnp.bfloat16
    u32 = jnp.uint32

    nsem = [0]

    def copy(src, dst):
        nsem[0] += 1
        return pltpu.make_async_copy(src, dst, sems.at[nsem[0] - 1])

    def piece(pc):
        if pc[0] == "x":
            _, j, b0, b1 = pc
            rows = pl.ds(b0 * C, (b1 - b0) * C)
            return [copy(x_hbm.at[0, rows, pl.ds(j * 128, 128)], x_vm.at[j, rows, :])]
        if pc[0] == "w":
            _, kk, t0, t1 = pc
            rows, cols = pl.ds(kk * 128, 128), pl.ds(t0 * D, (t1 - t0) * D)
            return [copy(w_hbm.at[rows, cols], w_raw.at[rows, cols])]
        if pc[0] == "wo":
            return [copy(wo_hbm.at[:, pl.ds(j * 128, 128)], wo_raw.at[j])
                    for j in range(LT)]
        if pc[0] == "vec":
            return [copy(wr_hbm, wr_vm), copy(gw_hbm, gw_vm)]
        assert pc[0] == "ffn"
        return [copy(wg_hbm, wg_vm), copy(wu_hbm, wu_vm), copy(wd_hbm, wd_vm)]

    stages = _stages(cfg)
    stage_cps = [[cp for pc in sg[0] for cp in piece(pc)] for sg in stages]

    def out_copy(r0, r1):
        return [copy(out_vm.at[pl.ds(r0, r1 - r0), :], out_hbm.at[0, pl.ds(r0, r1 - r0), :])]

    def x_lhs(s0, k0, k1):
        cols = [pltpu.bitcast(x_vm[j, s0:s0 + C, :], u32) for j in range(k0, k1)]
        return pltpu.bitcast(cols[0] if len(cols) == 1 else jnp.concatenate(cols, axis=1), bf16)

    def wait(cps, name):
        if cfg.get("scopes"):
            with jax.named_scope("wait_" + name):
                for cp in cps:
                    cp.wait()
        else:
            for cp in cps:
                cp.wait()

    for cps in stage_cps:
        for cp in cps:
            cp.start()

    qkv[LT:3 * LT, 0:HALO, :] = jnp.zeros((2 * LT, HALO, 128), f32)
    tscr[:, :, D // 2:, :] = jnp.zeros((LT, 3, 16, 128), u32)
    wo_u32[:, D // 2:, :] = jnp.zeros((LT, 16, 128), u32)

    def permute_w(kk, t0, t1):
        for t in range(t0, t1):
            for c in range(LT):
                tile = w_raw[kk * 128:(kk + 1) * 128,
                             t * D + c * 128:t * D + (c + 1) * 128]
                tscr[kk, t, c * 64:(c + 1) * 64, :] = pltpu.bitcast(tile.T, u32)
        for t in range(t0, t1):
            for dp in range(DH // 2):
                a = tscr[kk, t, pl.ds(dp, 16, stride=DH // 2), :]
                b = tscr[kk, t, pl.ds(160 + dp, 16, stride=DH // 2), :]
                ev, od = _interleave(a, b)
                r0 = (t * D + 2 * dp * 32) // 2
                wp[r0:r0 + 16, kk * 128:(kk + 1) * 128] = ev
                wp[r0 + 16:r0 + 32, kk * 128:(kk + 1) * 128] = od

    def permute_wo(c):
        wo_u32[c, 0:D // 2, :] = pltpu.bitcast(wo_raw[c], u32)
        outs = []
        for dp in range(DH // 2):
            a = wo_u32[c, pl.ds(dp, 16, stride=DH // 2), :]
            b = wo_u32[c, pl.ds(160 + dp, 16, stride=DH // 2), :]
            ev, od = _interleave(a, b)
            r0 = dp * 32
            wo_p[r0:r0 + 16, c * 128:(c + 1) * 128] = ev
            wo_p[r0 + 16:r0 + 32, c * 128:(c + 1) * 128] = od
            outs.append((ev, od))
        return outs

    wait(stage_cps[0], "s0")

    def tiles8(v):
        return [jnp.broadcast_to(v[:, j * 128:(j + 1) * 128], (8, 128)) for j in range(LT)]

    wr = gw = zvec = z16 = None

    def load_vectors():
        nonlocal wr, gw, zvec, z16
        wr = tiles8(wr_vm[...].astype(f32)[None, :])
        gw = tiles8(gw_vm[...].astype(f32)[None, :])
        zero = jax.lax.shift_right_logical(
            jnp.max(jax.lax.shift_right_logical(pltpu.bitcast(wr[0], jnp.int32), 16)), 16)
        zvec = pltpu.bitcast(jnp.full((8, 128), zero, jnp.int32), u32)
        z16 = pl.multiple_of(zero * 16, 16)

    def bits(v):
        return v if v.dtype == u32 else pltpu.bitcast(v, u32)

    def token(deps):
        u = None
        for d in deps:
            d = bits(d)
            for r in range(0, d.shape[0], 8):
                part = d if d.shape[0] == 8 else d[r:r + 8]
                u = part if u is None else u | part
        return u & zvec

    def tied(v, deps):
        if not deps:
            return v
        w = bits(v) | token(deps)
        return w if v.dtype == u32 else pltpu.bitcast(w, v.dtype)

    def load_tiles(ref, g0, g1, c0, c1, deps):
        lanes = slice(c0 * 128, c1 * 128)
        rows = sorted({g * 64 + 8 * deps[(g, c)][0] for g in range(g0, g1)
                       for c in range(c0, c1) if (g, c) in deps})
        parts, prev = [], g0 * 64
        for r in rows:
            if r > prev:
                parts.append(ref[prev:r, lanes])
            cols = []
            for c in range(c0, c1):
                pos, vals = deps.get((r // 64, c), (None, None))
                cols.append(tied(ref[r:r + 8, c * 128:(c + 1) * 128],
                                 vals if pos == (r % 64) // 8 else None))
            parts.append(cols[0] if len(cols) == 1 else jnp.concatenate(cols, axis=1))
            prev = r + 8
        if prev < g1 * 64:
            parts.append(ref[prev:g1 * 64, lanes])
        w = parts[0] if len(parts) == 1 else jnp.concatenate(parts, axis=0)
        return pltpu.bitcast(w, bf16)

    def unit_a(s0, xv, n0, n1, k0, k1, deps):
        w = load_tiles(wp, n0, n1, k0, k1, deps)
        y = jax.lax.dot_general(xv, w, _NT, preferred_element_type=f32)
        outs = []
        for j in range(n0, n1):
            blk = y[:, (j - n0) * 128:(j - n0 + 1) * 128]
            outs.append(blk)
            if k0 > 0:
                blk = blk + qkv[j, HALO + s0:HALO + s0 + C, :]
            qkv[j, HALO + s0:HALO + s0 + C, :] = blk
        return outs

    def unit_c(r0, n, moe, deps, per_tile_out=None):
        o = pltpu.bitcast(obuf[r0 // 2:(r0 + n) // 2, :], bf16)
        w = load_tiles(wo_p, 0, LT, 0, LT, deps)
        a = jnp.dot(o, w, preferred_element_type=f32)
        g = g_vm[r0:r0 + n, :]
        if moe is not None:
            idx, delta = moe
            hit = jax.lax.broadcasted_iota(jnp.int32, (n, 128), 0) + r0 == idx
        for j in range(LT):
            sl = slice(j * 128, (j + 1) * 128)
            x = x_vm[j, r0:r0 + n, :].astype(f32)
            if moe is not None:
                x = x + jnp.where(hit, delta[j], 0.0)
            res = x + g * (a[:, sl] - x)
            out_vm[r0:r0 + n, sl] = res.astype(bf16)
            if per_tile_out is not None and j in cfg["last_tiles"]:
                j0 = ([-1] + list(cfg["last_tiles"]))[cfg["last_tiles"].index(j)] + 1
                cols = pl.ds(j0 * 128, (j + 1 - j0) * 128)
                cp = copy(out_vm.at[pl.ds(r0, n), cols], out_hbm.at[0, pl.ds(r0, n), cols])
                cp.start()
                per_tile_out.append([cp])
        fence = pltpu.bitcast(out_vm[pl.ds(z16, 16), 0:128], u32)
        return [a[:, j * 128:(j + 1) * 128] for j in range(LT)], fence

    def attn_block(s0, rel):
        r0 = HALO + s0
        cq = tied(jnp.full((8, 128), CQ, f32), rel)
        q = qkv[0:LT, r0:r0 + R, :].reshape(LT * R // 8, 8, 128) * cq[None]
        q = q.reshape(LT, R, 128)
        ls = []
        for w in range(NW):
            rw = r0 - DIL * w
            s = jnp.sum(q * qkv[LT:2 * LT, rw:rw + R, :], axis=0)
            l = (s + pltpu.roll(s, 32, 1)) + (pltpu.roll(s, 64, 1) + pltpu.roll(s, 96, 1))
            if s0 < DIL * w:
                row = jax.lax.broadcasted_iota(jnp.int32, (R, 128), 0) + s0
                l = jnp.where(row >= DIL * w, l, NEG)
            ls.append(l)
        m = ls[0]
        for w in range(1, NW):
            m = jnp.maximum(m, ls[w])
        ps = [jnp.exp2(l - m) for l in ls]
        den = ps[0]
        for w in range(1, NW):
            den = den + ps[w]
        inv = pl.reciprocal(den, approx=True)
        inv = inv + inv * (1.0 - den * inv)
        o = ps[0][None] * qkv[2 * LT:3 * LT, r0:r0 + R, :]
        for w in range(1, NW):
            rw = r0 - DIL * w
            o = o + ps[w][None] * qkv[2 * LT:3 * LT, rw:rw + R, :]
        o = o * inv[None]
        outs = []
        for j in range(LT):
            oj = o[j]
            obuf[s0 // 2:(s0 + R) // 2, j * 128:(j + 1) * 128] = pltpu.bitcast(
                oj.astype(bf16), u32)
            outs.append(oj)
        return m, inv, outs

    def rowdot(mat, vec, stag=None):
        n = mat[0].shape[0]
        acc = None
        for j in range(LT):
            p = mat[j].reshape(n // 8, 8, 128) * vec[j][None]
            acc = p if acc is None else acc + p
        if stag is not None:
            acc = acc.reshape(len(stag), n // 8 // len(stag), 8, 128)
            acc = pltpu.bitcast(pltpu.bitcast(acc, u32) | stag[:, None], f32)
        acc = acc.reshape(n, 128)
        return jnp.broadcast_to(jnp.sum(acc, axis=-1, keepdims=True), (n, 128))

    def pre_block(b, racc, stag):
        lane = jax.lax.broadcasted_iota(jnp.int32, (PR, 128), 1)
        xf = [x_vm[j, b * PR:(b + 1) * PR, :].astype(f32) for j in range(LT)]
        g_vm[b * PR:(b + 1) * PR, :] = _sigmoid(rowdot(xf, gw, stag))
        return jnp.where(lane == b, rowdot(xf, wr, stag), racc)

    def ffn_block(b, xsel, yacc, stag):
        f0 = b * FB
        wg = wg_vm[f0:f0 + FB, :].astype(f32)
        wu = wu_vm[f0:f0 + FB, :].astype(f32)
        gt = rowdot([wg[:, j * 128:(j + 1) * 128] for j in range(LT)], xsel, stag)
        up = rowdot([wu[:, j * 128:(j + 1) * 128] for j in range(LT)], xsel, stag)
        h = gt * _sigmoid(gt) * up
        new = []
        for j in range(LT):
            p = wd_vm[f0:f0 + FB, j * 128:(j + 1) * 128].astype(f32) * h
            new.append(yacc[j] + jnp.sum(p.reshape(FB // 8, 8, 128), axis=0))
        return new

    def fence_g():
        return g_vm[pl.ds(z16, 8), :]

    nfb = F // FB
    npb = S // PR
    st = dict(
        now=0.0, busy=1e9, last_side=False,
        a_row=0, b_row=0, c_row=0, p=0, f=0, w=0,
        x_avail=0, wo_avail=False, until=None,
        qkv_ready=[(0, -1e9)],
        b_ready=[(0, -1e9)],
        slot_out=[],
        due=[],
        ffn_from=None, rtime=0.0,
        racc=jnp.full((PR, 128), -jnp.inf, f32),
        xsel=None, yacc=None, moe=None,
    )

    def avail(lst, t):
        return max(r for r, u in lst if u <= t)

    def barrier(copies, until=None, items=True):
        for cp, name in copies:
            wait(cp, name)
        st["slot_out"] = []
        st["due"] = []
        st["busy"] = st["now"] + cfg["first"] if items else 1e9
        st["until"] = until
        st["nxt"] = st["now"]
        st["pass"] = 0

    def place_item(t):
        if t < st["busy"]:
            return
        if st["until"] is not None and t >= st["until"] - cfg["quiet"]:
            return
        want = st["rtime"] - cfg["gap_r"]
        cand = [(rd, v) for (rd, v) in st["slot_out"] if rd <= want + 1e-6]

        def rel():
            if not cand:
                return []
            rd, v = cand[-1]
            r = min(v.shape[0] // 8 - 1, int((want - rd) * 16 + cfg["rel_row"] + 1e-6))
            return [v[8 * r:8 * r + 8]]

        def stag():
            if not cand:
                return None
            v, ng = cand[-1][1], cfg["stagger"]
            return bits(v.reshape(ng, v.shape[0] // 8 // ng, 8, 128)[:, 0]) & zvec[None]

        due = st["due"]
        can_p = st["p"] * PR < st["x_avail"]
        can_w = st["wo_avail"] and st["w"] < LT
        can_f = st["ffn_from"] is not None and t >= st["ffn_from"] and st["f"] < nfb
        p_urgent = st["p"] * PR < min(st["x_avail"], st["b_row"] + cfg["p_ahead"])
        b_urgent = st["a_row"] - st["b_row"] > cfg["b_behind"] and not can_w
        take_b = (st["b_row"] + R <= avail(st["qkv_ready"], t - cfg["b_slack"])
                  and not p_urgent
                  and (b_urgent or st["last_side"] or not (can_p or can_w or can_f)))
        st["last_side"] = not take_b
        if take_b:
            m, inv, obs = attn_block(st["b_row"], rel())
            due.append((t, m))
            due.append((t, inv))
            for j, ob in enumerate(obs):
                due.append((t + cfg["pv_off"][j], ob))
            st["b_row"] += R
            st["b_ready"].append((st["b_row"], t + cfg["pv_off"][-1] + 0.2))
            width = cfg["w_b"]
        elif can_w and not p_urgent:
            for dp, (ev, od) in enumerate(permute_wo(st["w"])):
                due.append((t + dp * cfg["s_w"], ev))
                due.append((t + dp * cfg["s_w"], od))
            st["w"] += 1
            width = cfg["w_w"]
        elif can_p:
            st["racc"] = pre_block(st["p"], st["racc"], stag())
            for u in range(PR // 8):
                due.append((t + u * 0.1, st["racc"][u * 8:(u + 1) * 8]))
            due.append((t + 0.8, fence_g()))
            st["p"] += 1
            width = cfg["w_p"]
        elif can_f:
            st["yacc"] = ffn_block(st["f"], st["xsel"], st["yacc"], stag())
            for j in range(LT):
                due.append((t + cfg["f_off"][j], st["yacc"][j]))
            st["f"] += 1
            width = cfg["w_f"]
        else:
            st["last_side"] = False
            return
        st["busy"] = max(st["busy"], t - 0.79) + width - 1e-6

    def plan_unit(passes, dur):
        deps = {}
        t0 = st["now"]
        st["pass_round"] = []
        for i, tile in enumerate(passes):
            t = t0 + i * dur
            if st["pass"] % 4 == 0:
                st["rtime"] = t / 0.8
            st["pass_round"].append(st["rtime"])
            if t >= st["nxt"] - 1e-6:
                place_item(t)
                st["nxt"] = t + 4 * dur
            vals = [v for (u, v) in st["due"] if u <= t + 1e-6]
            st["due"] = [(u, v) for (u, v) in st["due"] if u > t + 1e-6]
            if vals:
                deps[tile] = (cfg["pos"][st["pass"] % 4], vals)
            st["pass"] += 1
        st["now"] = t0 + len(passes) * dur
        return deps

    def run_a(s0, xv, n0, n1, k0, k1):
        deps = plan_unit([(n, kk) for n in range(n0, n1) for kk in range(k0, k1)], 1.0 / LT)
        outs = unit_a(s0, xv, n0, n1, k0, k1, deps)
        st["slot_out"] += [(st["pass_round"][(j + 1) * (k1 - k0) - 1], v)
                           for j, v in enumerate(outs)]

    kdone = [[0] * 3 for _ in range(S // C)]
    xhave = [0] * LT
    whave = set()

    def part(b, k1, t0=0, t1=3, hook=None):
        xvs = {}
        for t in range(t0, t1):
            k0 = kdone[b][t]
            if k0 >= k1:
                continue
            assert all(xhave[j] > b and (j, t) in whave for j in range(k0, k1)), (b, t, k1)
            if (b, t, k1) in cfg["halves"]:
                assert (k0, k1) == (0, 1)
                w = load_tiles(wp, t * LT, (t + 1) * LT, k0, k1, {})
                for s0 in (b * C, b * C + C // 2):
                    y = jax.lax.dot_general(x_vm[0, s0:s0 + C // 2, :], w, _NT,
                                            preferred_element_type=f32)
                    for j in range(LT):
                        qkv[t * LT + j, HALO + s0:HALO + s0 + C // 2, :] = (
                            y[:, j * 128:(j + 1) * 128])
                st["now"] += 1.0
                kdone[b][t] = k1
                continue
            if k0 not in xvs:
                xvs[k0] = x_lhs(b * C, k0, k1)
            xv = xvs[k0]
            grp = max(1, cfg["a_passes"] // (k1 - k0))
            for n0 in range(t * LT, (t + 1) * LT, grp):
                if hook is not None:
                    hook()
                run_a(b * C, xv, n0, min((t + 1) * LT, n0 + grp), k0, k1)
            kdone[b][t] = k1
        if min(kdone[b]) == LT:
            assert st["a_row"] == b * C
            st["a_row"] += C
            st["qkv_ready"].append((st["a_row"], st["now"]))

    def enter_stage(n, **kw):
        barrier([(stage_cps[n], "s%d" % n)] if n else [], **kw)
        for pc in stages[n][0]:
            if pc[0] == "x":
                assert xhave[pc[1]] == pc[2]
                xhave[pc[1]] = pc[3]
            elif pc[0] == "w":
                permute_w(*pc[1:])
                whave.update((pc[1], t) for t in range(pc[2], pc[3]))
            elif pc[0] == "wo":
                st["wo_avail"] = True
            elif pc[0] == "vec":
                load_vectors()
        st["x_avail"] = min(xhave) * C
        if any(pc[0] == "w" for pc in stages[n][0]):
            st["busy"] += cfg["first_perm"]
        for pt in stages[n][1]:
            part(*pt)

    n_main = len(stages) - 2
    for n in range(n_main):
        k_sim = [list(k) for k in kdone]
        length = 0
        for pt in stages[n][1]:
            b, k1, t0, t1 = (tuple(pt) + (0, 3))[:4]
            for t in range(t0, t1):
                length += max(0, k1 - k_sim[b][t])
                k_sim[b][t] = max(k1, k_sim[b][t])
        enter_stage(n, items=(n == n_main - 1), until=st["now"] + length)
    t_main = st["now"]
    enter_stage(n_main, until=t_main + cfg["late_t"])

    idx = r_sel = tile0 = None
    out_copies = []
    out_done = 0

    def moe_steps():
        nonlocal idx, r_sel, tile0, out_done
        if st["p"] == npb and idx is None:
            rb = st["racc"].astype(bf16).astype(f32)
            rb = jnp.where(rb != rb, -jnp.inf, rb)
            rmax = jnp.max(rb)
            rowid = (jax.lax.broadcasted_iota(jnp.int32, (PR, 128), 1) * PR
                     + jax.lax.broadcasted_iota(jnp.int32, (PR, 128), 0))
            idx = jnp.min(jnp.where((rowid < S) & (rb == rmax), rowid, S - 1))
            tile0 = pl.multiple_of((idx // 16) * 16, 16)
            r_sel = _sigmoid(jnp.full((1, 128), rmax, f32))
            row16 = jax.lax.broadcasted_iota(jnp.int32, (16, 128), 0) + tile0
            st["xsel"] = [
                jnp.broadcast_to(jnp.sum(
                    jnp.where(row16 == idx,
                              x_vm[j, pl.ds(tile0, 16), :].astype(f32), 0.0),
                    axis=0, keepdims=True), (8, 128)) for j in range(LT)]
            st["yacc"] = [jnp.zeros((8, 128), f32) for _ in range(LT)]
            st["ffn_from"] = st["now"] + cfg["router_gap"]
        elif st["f"] == nfb and st["moe"] is None:
            delta = [jnp.sum(y, axis=0, keepdims=True) * r_sel for y in st["yacc"]]
            st["moe"] = (idx, delta)
            fix_rows = st["c_row"]
            t0 = pl.multiple_of(jnp.minimum(tile0, fix_rows - 16), 16)
            row = jax.lax.broadcasted_iota(jnp.int32, (16, 128), 0) + t0
            coef = 1.0 - g_vm[pl.ds(t0, 16), :]
            cur = out_vm[pl.ds(t0, 16), :].astype(f32)
            upd = jnp.concatenate(
                [jnp.where(row == idx, coef * delta[j], 0.0) for j in range(LT)], axis=1)
            out_vm[pl.ds(t0, 16), :] = (cur + upd).astype(bf16)
            cp = out_copy(0, fix_rows)
            cp[0].start()
            out_copies.append(cp)
            out_done = fix_rows

    def late_barrier():
        if (st["x_avail"] < S and st["now"] >= t_main + cfg["late_t"] - 1e-6
                and (st["pass"] % 4 == 0 or st["now"] >= t_main + cfg["late_t"] + 4)):
            if cfg.get("verbose"):
                print("late barrier at", st["now"] - t_main, "pass", st["pass"])
            enter_stage(n_main + 1)

    while st["c_row"] < S:
        late_barrier()
        a_row, c_row = st["a_row"], st["c_row"]
        cc = cfg["CC"] if c_row < S - cfg["tail_rows"] else cfg["tail_cc"]
        c_ok = (avail(st["b_ready"], st["now"] - cfg["c_slack"]) >= c_row + cc
                and st["p"] * PR >= c_row + cc and st["w"] == LT)
        units = []
        if a_row < S and (not c_ok or a_row - c_row < cfg["c_lag"]):
            units = ["a"]
        elif c_ok:
            units = ["c"]
        else:
            place_item(st["now"])
            st["due"] = []
            st["now"] += 1.0
        for kind in units:
            if kind == "a":
                part(a_row // C, LT, hook=lambda: (late_barrier(), moe_steps()))
            else:
                dur = cc / C
                deps = plan_unit([(kk, n) for n in range(LT) for kk in range(LT)], dur / LT)
                split = cfg["last_tiles"] and c_row + cc == S and out_done == c_row
                outs, fence = unit_c(c_row, cc, st["moe"], deps,
                                      out_copies if split else None)
                if split:
                    out_done = S
                st["slot_out"] += [(st["pass_round"][(j + 1) * LT - 1], v)
                                   for j, v in enumerate(outs)]
                st["c_row"] += cc
                st["due"].append((st["now"] + cfg["fence_lag"], fence))
                st["busy"] = max(st["busy"], st["now"] - 1)
                if st["moe"] is not None and out_done < S and (
                        st["c_row"] in cfg["out_splits"] or st["c_row"] == S):
                    cp = out_copy(out_done, st["c_row"])
                    cp[0].start()
                    out_copies.append(cp)
                    out_done = st["c_row"]
            moe_steps()
        if cfg.get("verbose"):
            print(round(st["now"] - t_main, 1),
                  {k: st[k] for k in ("a_row", "b_row", "c_row", "p", "f", "w")})

    assert out_done == S
    for n, cp in enumerate(out_copies):
        wait(cp, "o%d" % n)


def _kernel_once(*refs, cfg):
    pl.when(pl.program_id(0) == 0)(lambda: _kernel(*refs, cfg=cfg))


def _build(cfg):
    bf16 = jnp.bfloat16
    f32 = jnp.float32
    u32 = jnp.uint32
    hbm_spec = pl.BlockSpec(memory_space=pltpu.MemorySpace.HBM)
    no_checks = {k: True for k in ("disable_bounds_checks", "disable_semaphore_checks")
                 if hasattr(pltpu.CompilerParams, k)}
    return pl.pallas_call(
        functools.partial(_kernel_once, cfg=cfg),
        grid=(2,),
        out_shape=jax.ShapeDtypeStruct((1, S, D), bf16),
        in_specs=[hbm_spec] * 8,
        out_specs=hbm_spec,
        scratch_shapes=[
            pltpu.VMEM((LT, S, 128), bf16),
            pltpu.VMEM((D, 3 * D), bf16),
            pltpu.VMEM((LT, 3, D // 2 + 16, 128), u32),
            pltpu.VMEM((3 * D // 2, D), u32),
            pltpu.VMEM((LT, D, 128), bf16),
            pltpu.VMEM((LT, D // 2 + 16, 128), u32),
            pltpu.VMEM((D // 2, D), u32),
            pltpu.VMEM((D,), bf16),
            pltpu.VMEM((D,), bf16),
            pltpu.VMEM((F, D), bf16),
            pltpu.VMEM((F, D), bf16),
            pltpu.VMEM((F, D), bf16),
            pltpu.VMEM((3 * LT, HALO + S, 128), f32),
            pltpu.VMEM((S // 2, D), u32),
            pltpu.VMEM((S, D), bf16),
            pltpu.VMEM((S, 128), f32),
            pltpu.SemaphoreType.DMA((48 + len(cfg["out_splits"]),)),
        ],
        compiler_params=pltpu.CompilerParams(
            dimension_semantics=("arbitrary",),
            vmem_limit_bytes=100 * 1024 * 1024,
            **no_checks),
    )


def _call(cfg, A_x, A_wqkv, A_wo, B_w_r, B_w_gate, B_w_up, B_w_down, gate_w):
    return _build(cfg)(A_x, A_wqkv, A_wo, B_w_r, B_w_gate.T, B_w_up.T, B_w_down, gate_w)


@jax.jit
def pallas_gated_mix__sliding_local_dilated__moe_arch_mod__prompt_kernel(
    A_x: jax.Array,
    A_wqkv: jax.Array,
    A_wo: jax.Array,
    B_x: jax.Array,
    B_w_r: jax.Array,
    B_w_gate: jax.Array,
    B_w_up: jax.Array,
    B_w_down: jax.Array,
    gate_w: jax.Array,
):
    del B_x
    return _call(CFG, A_x, A_wqkv, A_wo, B_w_r, B_w_gate, B_w_up, B_w_down, gate_w)
```
